```python
import jax
import jax.numpy as jnp

def _softmax(x, axis=-1):
    return jax.nn.softmax(x, axis=axis)
def _gelu(x):
    return jax.nn.gelu(x, approximate=True)
def _silu(x):
    return jax.nn.silu(x)
def _sigmoid(x):
    return jax.nn.sigmoid(x)
def _layernorm(x, axis=-1, eps=1e-5):
    m = jnp.mean(x, axis=axis, keepdims=True)
    v = jnp.var(x, axis=axis, keepdims=True)
    return (x - m) / jnp.sqrt(v + eps)
def _scatter_add(tgt, idx, src, axis=0):
    return tgt.at[idx].add(src)
def _segment_sum(src, seg, n):
    return jax.ops.segment_sum(src, seg, n)
class _Rng:
    def __init__(self, key):
        self._k = key
    def _next(self):
        self._k, sub = jax.random.split(self._k)
        return sub
    def normal(self, shape):
        return jax.random.normal(self._next(), shape, dtype=jnp.bfloat16)
    def randint(self, lo, hi, shape):
        return jax.random.randint(self._next(), shape, lo, hi, dtype=jnp.int32)
    def uniform(self, shape, lo=0.0, hi=1.0):
        return jax.random.uniform(self._next(), shape, jnp.bfloat16, lo, hi)
    def permutation(self, n):
        return jax.random.permutation(self._next(), n)


kernel_name = 'concat_heads__compressed_kv_cla__mha_block_cached__decode'

def setup_inputs():
    _rng = _Rng(jax.random.key(int.from_bytes(__import__("os").urandom(4), "little")))
    _w = (lambda a: (lambda t: t.astype(jnp.bfloat16) if jnp.issubdtype(t.dtype, jnp.floating) else t)(jnp.asarray(a)))
    def _A_setup():
        B, H, Sq, Sk, D, M = 4, 32, 1, 4096, 128, 512
        Dc = 4 * D
        return {
            "x": _w((lambda *s: _rng.normal(s) * 0.05)(B, Sq, M)),
            "c_kv": _w((lambda *s: _rng.normal(s) * 0.05)(B, Sk, Dc)),
            "w_q": _w((lambda *s: _rng.normal(s) * 0.05)(M, H, D) * (M ** -0.5)),
            "w_uk": _w((lambda *s: _rng.normal(s) * 0.05)(Dc, H, D) * (Dc ** -0.5)),
            "w_uv": _w((lambda *s: _rng.normal(s) * 0.05)(Dc, H, D) * (Dc ** -0.5)),
            "w_o": _w((lambda *s: _rng.normal(s) * 0.05)(H, D, M) * ((H * D) ** -0.5)),
        }
    _A_in = _A_setup()

    def _B_setup():
        B, Sq, D = 4, 1, 512
        H, Sk, Dh = 32, 4096, 128
        return {
            "x": _w((lambda *s: _rng.normal(s) * 0.05)(B, Sq, D)),
            "k_cache": _w((lambda *s: _rng.normal(s) * 0.05)(B, H, Sk, Dh)),
            "v_cache": _w((lambda *s: _rng.normal(s) * 0.05)(B, H, Sk, Dh)),
            "wq": _w((lambda *s: _rng.normal(s) * 0.05)(D, H * Dh) * (D ** -0.5)),
            "wo": _w((lambda *s: _rng.normal(s) * 0.05)(H * Dh, D) * ((H * Dh) ** -0.5)),
        }
    _B_in = _B_setup()

    return {
        "A_x": _A_in["x"],
        "A_c_kv": _A_in["c_kv"],
        "A_w_q": _A_in["w_q"],
        "A_w_uk": _A_in["w_uk"],
        "A_w_uv": _A_in["w_uv"],
        "A_w_o": _A_in["w_o"],
        "B_x": _B_in["x"],
        "B_k_cache": _B_in["k_cache"],
        "B_v_cache": _B_in["v_cache"],
        "B_wq": _B_in["wq"],
        "B_wo": _B_in["wo"],
    }

def reference(A_x, A_c_kv, A_w_q, A_w_uk, A_w_uv, A_w_o, B_x, B_k_cache, B_v_cache, B_wq, B_wo):
    def _A_ref(x, c_kv, w_q, w_uk, w_uv, w_o):
        B, Sq, M = x.shape[0], x.shape[1], x.shape[2]
        Sk = c_kv.shape[1]
        H, D = w_q.shape[1], w_q.shape[2]
        q = jnp.einsum("bqm,mhd->bhqd", x, w_q)
        k = jnp.einsum("bkc,chd->bhkd", c_kv, w_uk)
        v = jnp.einsum("bkc,chd->bhkd", c_kv, w_uv)
        scores = jnp.einsum("bhqd,bhkd->bhqk", q, k) * (D ** -0.5)
        off = Sk - Sq
        qi = jnp.arange(Sq)[:, None]
        kj = jnp.arange(Sk)[None, :]
        cmask = kj <= (qi + off)
        scores = jnp.where(cmask[None, None], scores, -1e9)
        p = _softmax(scores, axis=-1)
        ctx = jnp.einsum("bhqk,bhkd->bhqd", p, v)
        return jnp.einsum("bhqd,hdm->bqm", ctx, w_o)

    def _B_ref(x, k_cache, v_cache, wq, wo):
        B, Sq, D = x.shape
        H, Dh = 32, 128
        q = (lambda x, *d: x.transpose(*d))((x @ wq).reshape(B, Sq, H, Dh), 0, 2, 1, 3)
        scores = jnp.einsum("bhqd,bhkd->bhqk", q, k_cache) * (Dh ** -0.5)
        p = _softmax(scores, axis=-1)
        o = jnp.einsum("bhqk,bhkd->bhqd", p, v_cache)
        return (lambda x, *d: x.transpose(*d))(o, 0, 2, 1, 3).reshape(B, Sq, H * Dh) @ wo

    a = _A_ref(A_x, A_c_kv, A_w_q, A_w_uk, A_w_uv, A_w_o)
    b = _B_ref(B_x, B_k_cache, B_v_cache, B_wq, B_wo)
    return jnp.concatenate([a, b], axis=-1)
```

```python
import functools

import jax
import jax.numpy as jnp
from jax import lax
import jax.experimental.pallas as pl
import jax.experimental.pallas.tpu as pltpu

B, H, SK, D, M = 4, 32, 4096, 128, 512
DC = 512
NSTEPS = B * H
NSLOT = 4
F32 = jnp.float32
BF16 = jnp.bfloat16
LO, HI = 1, 0


def _dot(a, b):
    return jnp.dot(a, b, preferred_element_type=F32)


def _dot_nt(a, b):
    return lax.dot_general(a, b, (((1,), (1,)), ((), ())), preferred_element_type=F32)


def make_kernel(LROWS=256, HROWS=128, NVL=9, NEX=10, DL=2, compute=True, acompute=True, pace=True):
    NK = SK // LROWS
    VL_ROWS = NVL * LROWS
    NVH = (SK - VL_ROWS) // HROWS
    NPTS = NK + NVL
    assert NVH + NEX <= NPTS
    scale = D ** -0.5
    EX = [("wqa", 128), ("wuk", 128), ("ckv", 512), ("wuv", 128), ("woa", 128), ("wob", 128)]
    ex_start = {}
    tot = 0
    for name, n in EX:
        ex_start[name] = tot
        tot += n
    EX_TOTAL = tot

    def ready_step(name, upto=None):
        n = dict(EX)[name] if upto is None else upto
        last = ex_start[name] + n - 1
        return last // NEX + 2

    def kernel(xa_h, ckv_h, wqa_h, wuk_h, wuv_h, woa_h, xb_h, k_h, v_h, wqb_h, wob_h,
               out_ref,
               kbuf, vbuf, wqb_v, wqa_v, wuk_v, wuv_v, ckv_v, woa_v, wob_v, xa_v, xb_v,
               xs, qb_s, o_s, qa_s, qabs_s, s_s, p_s, l_s, acc_s, ctxc_s, ctx_s, outa_s, outb_s,
               lsem, hsem, esem, xsem):

        def bh(i):
            return i & (B - 1), i >> 2

        def k_chunk(i, j):
            b, h = bh(i)
            r = j * LROWS
            slot = i & (NSLOT - 1)
            return pltpu.make_async_copy(k_h.at[b, h, pl.ds(r, LROWS)], kbuf.at[slot, pl.ds(r, LROWS)],
                                         lsem.at[slot * NPTS + j])

        def vl_chunk(i, j):
            b, h = bh(i)
            r = j * LROWS
            slot = i & (NSLOT - 1)
            return pltpu.make_async_copy(v_h.at[b, h, pl.ds(r, LROWS)], vbuf.at[slot, pl.ds(r, LROWS)],
                                         lsem.at[slot * NPTS + NK + j])

        def vh_chunk(i, j):
            b, h = bh(i)
            r = VL_ROWS + j * HROWS
            slot = i & (NSLOT - 1)
            return pltpu.make_async_copy(v_h.at[b, h, pl.ds(r, HROWS)], vbuf.at[slot, pl.ds(r, HROWS)],
                                         hsem.at[slot])

        def vh_all(i):
            b, h = bh(i)
            slot = i & (NSLOT - 1)
            n = SK - VL_ROWS
            return pltpu.make_async_copy(v_h.at[b, h, pl.ds(VL_ROWS, n)], vbuf.at[slot, pl.ds(VL_ROWS, n)],
                                         hsem.at[slot])

        def issue_extra(e):
            def rng(name):
                s = ex_start[name]
                return jnp.logical_and(e >= s, e < s + dict(EX)[name])

            for idx, (name, src, dst) in enumerate((("wqa", wqa_h, wqa_v), ("wuk", wuk_h, wuk_v),
                                                    ("wuv", wuv_h, wuv_v))):
                @pl.when(rng(name))
                def _():
                    r = (e - ex_start[name]) * 4
                    pltpu.make_async_copy(src.at[pl.ds(r, 4)], dst.at[pl.ds(r, 4)], esem.at[idx]).start(priority=HI)

            @pl.when(rng("ckv"))
            def _():
                c = e - ex_start["ckv"]
                b = c >> 7
                r = pl.multiple_of((c & 127) * 32, 32)
                pltpu.make_async_copy(ckv_h.at[b, pl.ds(r, 32)], ckv_v.at[b, pl.ds(r, 32)],
                                      esem.at[3 + b]).start(priority=HI)

            @pl.when(rng("woa"))
            def _():
                c = e - ex_start["woa"]
                h = c >> 2
                r = pl.multiple_of((c & 3) * 32, 32)
                pltpu.make_async_copy(woa_h.at[h, pl.ds(r, 32)], woa_v.at[h, pl.ds(r, 32)],
                                      esem.at[7]).start(priority=HI)

            @pl.when(rng("wob"))
            def _():
                c = e - ex_start["wob"]
                r = pl.multiple_of(c * 32, 32)
                pltpu.make_async_copy(wob_h.at[pl.ds(r, 32)], wob_v.at[pl.ds(r, 32)],
                                      esem.at[8]).start(priority=HI)

        def issue_h(i, p, last):
            if last:
                return
            if p < NVH:
                vh_chunk(i + 1, p).start(priority=HI)
            elif p < NVH + NEX:
                issue_extra(i * NEX + (p - NVH))

        wqb_cp = pltpu.make_async_copy(wqb_h, wqb_v, xsem.at[0])
        wqb_cp.start(priority=HI)
        xb_cp = pltpu.make_async_copy(xb_h, xb_v, xsem.at[1])
        xb_cp.start(priority=HI)
        xa_cp = pltpu.make_async_copy(xa_h, xa_v, xsem.at[2])
        xa_cp.start(priority=HI)
        vh_all(0).start(priority=HI)
        for s in range(DL):
            for j in range(NK):
                k_chunk(s, j).start(priority=LO)
            for j in range(NVL):
                vl_chunk(s, j).start(priority=LO)

        o_s[...] = jnp.zeros(o_s.shape, F32)
        xs[...] = jnp.zeros(xs.shape, F32)
        xb_cp.wait()
        xa_cp.wait()
        xs[0, 0:B, :] = xa_v[...].astype(F32)
        xs[1, 0:B, :] = xb_v[...].astype(F32)
        wqb_cp.wait()
        qb = _dot(xs[1].astype(BF16), wqb_v[...])
        for h in range(H):
            qb_s[h] = qb[:, h * D:(h + 1) * D]

        row8 = lax.broadcasted_iota(jnp.int32, (8, D), 0)

        S_QA = ready_step("wqa")
        S_QABS = max(ready_step("wuk"), S_QA + 4)
        S_ATT = max(ready_step("ckv", 128), S_QABS + 4)
        ATT_STRIDE = 13
        assert all(S_ATT + b * ATT_STRIDE >= ready_step("ckv", 128 * (b + 1)) for b in range(B))
        S_CTX = max(ready_step("wuv"), S_ATT + 3 * ATT_STRIDE + 8)
        S_OUTA = max(ready_step("woa"), S_CTX + 4)
        S_OUTB = NSTEPS - B
        assert S_OUTB >= ready_step("wob") and S_OUTA < S_OUTB
        HG = 8

        def a_work(i):
            @pl.when(i == S_QA)
            def _():
                pltpu.make_async_copy(wqa_h, wqa_v, esem.at[0]).wait()

            for g in range(H // HG):
                @pl.when(i == S_QA + g)
                def _():
                    wt = jnp.swapaxes(wqa_v[:, g * HG:(g + 1) * HG, :], 0, 1)
                    x = xs[0].astype(BF16)
                    for hh in range(HG):
                        qa_s[g * HG + hh] = _dot(x, wt[hh])

            @pl.when(i == S_QABS)
            def _():
                pltpu.make_async_copy(wuk_h, wuk_v, esem.at[1]).wait()

            for g in range(H // HG):
                @pl.when(i == S_QABS + g)
                def _():
                    wt = jnp.swapaxes(wuk_v[:, g * HG:(g + 1) * HG, :], 0, 1)
                    t = jnp.stack([_dot_nt(qa_s[g * HG + hh].astype(BF16), wt[hh]) for hh in range(HG)])
                    qabs_s[:, g * HG:(g + 1) * HG, :] = jnp.swapaxes(t, 0, 1)

            ia = i - S_ATT
            ab = ia // ATT_STRIDE
            ap = ia % ATT_STRIDE
            in_att = jnp.logical_and(ia >= 0, ab < B)
            CH = SK // 4

            @pl.when(jnp.logical_and(in_att, ap == 0))
            def _():
                pltpu.make_async_copy(ckv_h.at[ab], ckv_v.at[ab], esem.at[3 + ab]).wait()

            @pl.when(jnp.logical_and(in_att, ap < 4))
            def _():
                r = pl.multiple_of(ap * CH, CH)
                s_s[ap] = _dot_nt(qabs_s[ab].astype(BF16), ckv_v[ab, pl.ds(r, CH), :])

            @pl.when(jnp.logical_and(in_att, ap == 4))
            def _():
                s = s_s[...]
                m = jnp.max(jnp.max(s, axis=0), axis=-1, keepdims=True)
                p = jnp.exp((s - m[None]) * scale)
                l_s[...] = jnp.broadcast_to(jnp.sum(jnp.sum(p, axis=0), axis=-1, keepdims=True), l_s.shape)
                p_s[...] = p.astype(BF16)
                acc_s[...] = jnp.zeros(acc_s.shape, F32)

            @pl.when(jnp.logical_and(in_att, jnp.logical_and(ap >= 4, ap < 8)))
            def _():
                t = ap - 4
                r = pl.multiple_of(t * CH, CH)
                acc_s[...] += _dot(p_s[t], ckv_v[ab, pl.ds(r, CH), :])

            @pl.when(jnp.logical_and(in_att, ap == 7))
            def _():
                ctxc_s[ab] = acc_s[...] / l_s[:, 0:1]

            @pl.when(i == S_CTX)
            def _():
                pltpu.make_async_copy(wuv_h, wuv_v, esem.at[2]).wait()

            for g in range(H // HG):
                @pl.when(i == S_CTX + g)
                def _():
                    wt = jnp.swapaxes(wuv_v[:, g * HG:(g + 1) * HG, :], 0, 1)
                    c = jnp.swapaxes(ctxc_s[:, g * HG:(g + 1) * HG, :], 0, 1)
                    for hh in range(HG):
                        ctx_s[g * HG + hh] = _dot(c[hh].astype(BF16), wt[hh])

            @pl.when(i == S_OUTA)
            def _():
                pltpu.make_async_copy(woa_h, woa_v, esem.at[7]).wait()
                c = jnp.concatenate([ctx_s[h] for h in range(H)], axis=-1).astype(BF16)
                outa_s[...] = _dot(c, woa_v[...].reshape(H * D, M))

            @pl.when(i == S_OUTB)
            def _():
                pltpu.make_async_copy(wob_h, wob_v, esem.at[8]).wait()
                c = jnp.concatenate([o_s[h] for h in range(H - 1)], axis=-1).astype(BF16)
                outb_s[...] = _dot(c, wob_v[0:(H - 1) * D, :])

        ctxc_s[...] = jnp.zeros(ctxc_s.shape, F32)

        def step(i, last):
            b, h = bh(i)
            slot = i & (NSLOT - 1)

            for j in range(NK):
                issue_h(i, j, last)
                k_chunk(i, j).wait()
                if not last:
                    @pl.when(i + DL < NSTEPS)
                    def _():
                        k_chunk(i + DL, j).start(priority=LO)

            if compute:
                q = qb_s[h].astype(BF16)
                s = _dot_nt(q, kbuf[slot])
                m = jnp.max(s, axis=-1, keepdims=True)
                p = jnp.exp((s - m) * scale)
                l = jnp.sum(p, axis=-1, keepdims=True)
                pb = p.astype(BF16)
            vh_all(i).wait()
            if compute:
                o = _dot(pb[:, VL_ROWS:], vbuf[slot, VL_ROWS:, :])

            if not last:
                for j in range(NVL):
                    issue_h(i, NK + j, last)
                    vl_chunk(i, j).wait()

                    @pl.when(i + DL < NSTEPS)
                    def _():
                        vl_chunk(i + DL, j).start(priority=LO)
                if compute:
                    o = o + _dot(pb[:, :VL_ROWS], vbuf[slot, :VL_ROWS, :])
            else:
                for j in range(NVL):
                    vl_chunk(i, j).wait()
                    if compute:
                        o = o + _dot(pb[:, j * LROWS:(j + 1) * LROWS], vbuf[slot, j * LROWS:(j + 1) * LROWS, :])
            if compute:
                o = jnp.where(row8 == b, o / l, o_s[h])
                if not last:
                    o_s[h] = o
                return o

        def body(i, c):
            step(i, False)
            if acompute:
                a_work(i)
            return c
        lax.fori_loop(0, NSTEPS - 1, body, 0)
        o = step(NSTEPS - 1, True)
        if not acompute:
            for idx, (src, dst) in enumerate(((wqa_h, wqa_v), (wuk_h, wuk_v), (wuv_h, wuv_v))):
                pltpu.make_async_copy(src, dst, esem.at[idx]).wait()
            for b in range(B):
                pltpu.make_async_copy(ckv_h.at[b], ckv_v.at[b], esem.at[3 + b]).wait()
            pltpu.make_async_copy(woa_h, woa_v, esem.at[7]).wait()
            pltpu.make_async_copy(wob_h, wob_v, esem.at[8]).wait()
        if compute:
            ob = outb_s[...] + _dot(o.astype(BF16), wob_v[(H - 1) * D:, :])
        else:
            ob = outb_s[...]
        res = jnp.concatenate([outa_s[...], ob], axis=-1)
        out_ref[...] = res[0:B, :].astype(out_ref.dtype)

    scratch = [
        pltpu.VMEM((NSLOT, SK, D), BF16), pltpu.VMEM((NSLOT, SK, D), BF16),
        pltpu.VMEM((M, H * D), BF16), pltpu.VMEM((M, H, D), BF16), pltpu.VMEM((DC, H, D), BF16),
        pltpu.VMEM((DC, H, D), BF16), pltpu.VMEM((B, SK, DC), BF16), pltpu.VMEM((H, D, M), BF16),
        pltpu.VMEM((H * D, M), BF16), pltpu.VMEM((B, M), BF16), pltpu.VMEM((B, M), BF16),
        pltpu.VMEM((2, 8, M), F32),
        pltpu.VMEM((H, 8, D), F32),
        pltpu.VMEM((H, 8, D), F32),
        pltpu.VMEM((H, 8, D), F32),
        pltpu.VMEM((8, H, DC), F32),
        pltpu.VMEM((4, H, SK // 4), F32),
        pltpu.VMEM((4, H, SK // 4), BF16),
        pltpu.VMEM((H, 128), F32),
        pltpu.VMEM((H, DC), F32),
        pltpu.VMEM((8, H, DC), F32),
        pltpu.VMEM((H, 8, D), F32),
        pltpu.VMEM((8, M), F32),
        pltpu.VMEM((8, M), F32),
        pltpu.SemaphoreType.DMA((NSLOT * NPTS,)),
        pltpu.SemaphoreType.DMA((NSLOT,)),
        pltpu.SemaphoreType.DMA((9,)),
        pltpu.SemaphoreType.DMA((3,)),
    ]

    @jax.jit
    def fn(A_x, A_c_kv, A_w_q, A_w_uk, A_w_uv, A_w_o, B_x, B_k_cache, B_v_cache, B_wq, B_wo):
        out = pl.pallas_call(
            kernel,
            in_specs=[pl.BlockSpec(memory_space=pl.ANY)] * 11,
            out_specs=pl.BlockSpec(memory_space=pltpu.VMEM),
            out_shape=jax.ShapeDtypeStruct((B, 2 * M), BF16),
            scratch_shapes=scratch,
            compiler_params=pltpu.CompilerParams(vmem_limit_bytes=100 * 1024 * 1024, disable_bounds_checks=True),
            name="fused_decode",
        )(A_x.reshape(B, M), A_c_kv, A_w_q, A_w_uk, A_w_uv, A_w_o, B_x.reshape(B, M), B_k_cache, B_v_cache, B_wq, B_wo)
        return out.reshape(B, 1, 2 * M)

    return fn


_fn = make_kernel()


@jax.jit
def pallas_concat_heads__compressed_kv_cla__mha_block_cached__decode_kernel(
    A_x: jax.Array,
    A_c_kv: jax.Array,
    A_w_q: jax.Array,
    A_w_uk: jax.Array,
    A_w_uv: jax.Array,
    A_w_o: jax.Array,
    B_x: jax.Array,
    B_k_cache: jax.Array,
    B_v_cache: jax.Array,
    B_wq: jax.Array,
    B_wo: jax.Array,
):
    return _fn(A_x, A_c_kv, A_w_q, A_w_uk, A_w_uv, A_w_o, B_x, B_k_cache, B_v_cache, B_wq, B_wo)
```

```python
import jax
import jax.numpy as jnp
from jax import lax
import jax.experimental.pallas as pl
import jax.experimental.pallas.tpu as pltpu

B, H, SK, D, M = 4, 32, 4096, 128, 512
DC = 512
HG = 8
NG = B * H // HG
F32 = jnp.float32
BF16 = jnp.bfloat16
LO, HI = 1, 0
NSEM = 48
SCALE = D ** -0.5


def _dot(a, b):
    return jnp.dot(a, b, preferred_element_type=F32)


def _dot_nt(a, b):
    return lax.dot_general(a, b, (((1,), (1,)), ((), ())), preferred_element_type=F32)


def _mo(x, n):
    return x if isinstance(x, int) else pl.multiple_of(x, n)


class _Rows:
    def __init__(self, src, dst, pat, hrows, ntr):
        self.src, self.dst, self.pat, self.hrows, self.ntr = src, dst, pat, hrows, ntr
        self.lrows = sum(pat) * ntr

    def lo(self, tr, k, sem):
        r = _mo(tr * sum(self.pat) + sum(self.pat[:k]), 8)
        n = self.pat[k]
        return pltpu.make_async_copy(self.src.at[:, pl.ds(r, n)], self.dst.at[:, pl.ds(r, n)], sem)

    def hi(self, tr, k, sem):
        r = _mo(self.lrows + (tr * 3 + k) * self.hrows, 8)
        n = self.hrows
        return pltpu.make_async_copy(self.src.at[:, pl.ds(r, n)], self.dst.at[:, pl.ds(r, n)], sem)

    def hi_span(self, r, n, sem):
        r = _mo(self.lrows + r, 8)
        return pltpu.make_async_copy(self.src.at[:, pl.ds(r, n)], self.dst.at[:, pl.ds(r, n)], sem)

    def hi_all(self, sem):
        return self.hi_span(0, self.hrows * 3 * self.ntr, sem)


class _Wide:
    ntr = 16
    hpat = (384, 384, 256)

    def __init__(self, src, dst):
        self.src, self.dst = src, dst

    def lo(self, tr, k, sem):
        c = tr * 3 + k
        r = _mo((c >> 2) * 8, 8)
        l = _mo((c & 3) * 1024, 128)
        idx = (slice(None), pl.ds(r, 8), pl.ds(l, 1024))
        return pltpu.make_async_copy(self.src.at[idx], self.dst.at[idx], sem)

    def hi(self, tr, k, sem):
        r = _mo(96 + (tr >> 2) * 8, 8)
        l = _mo((tr & 3) * 1024 + sum(self.hpat[:k]), 128)
        idx = (slice(None), pl.ds(r, 8), pl.ds(l, self.hpat[k]))
        return pltpu.make_async_copy(self.src.at[idx], self.dst.at[idx], sem)

    def hi_all(self, sem):
        idx = (slice(None), pl.ds(96, 32))
        return pltpu.make_async_copy(self.src.at[idx], self.dst.at[idx], sem)


def make_kernel(DT=12, compute=True, acompute=True):
    assert DT < 16

    def kernel(xa_h, ckv_h, wqa_h, wuk_h, wuv_h, woa_h, xb_h, k_h, v_h, wqb_h, wob_h,
               out_ref,
               kbuf, vbuf, wqb_v, wqa_v, wuk_v, wuv_v, ckv_v, woa_v, wob_v, xa_v, xb_v,
               xs, qb_s, qm_s, s_s, l_s, acc_s, o_s,
               qa_s, qabs_s, sa_s, pa_s, la_s, acca_s, ctxc_s, ctx_s, outb_s,
               lsem, hsem, esem, xsem):

        def n128(src, dst):
            return _Rows(src, dst, (48, 48, 64), 32, 16)

        def n512(src, dst):
            return _Rows(src, dst, (16, 16, 8), 8, 16)

        def kv(a, g):
            src = (k_h, v_h)[a].at[g & (B - 1), pl.ds((g >> 2) * HG, HG)]
            dst = (kbuf, vbuf)[a]
            return _Rows(src, dst, (24, 24, 32), 16, 32)

        def ckvb(b):
            return n512(ckv_h.at[pl.ds(b * 4, 4)], ckv_v.at[pl.ds(b * 4, 4)])

        wqb_b = _Wide(wqb_h, wqb_v)
        wqa_b, wuk_b, wuv_b = n128(wqa_h, wqa_v), n128(wuk_h, wuk_v), n128(wuv_h, wuv_v)
        woa_b, wob_b = n512(woa_h, woa_v), n512(wob_h, wob_v)

        def lsem_at(tr, k):
            return lsem.at[(tr & 15) * 3 + k]

        def point(cur, tr, k, hs, nxts):
            if hs is not None:
                cur.hi(tr, k, hs).start(priority=HI)
            cur.lo(tr, k, lsem_at(tr, k)).wait()
            ta = tr + DT
            sem = lsem_at(ta, k)
            if isinstance(tr, int):
                if ta < cur.ntr:
                    cur.lo(ta, k, sem).start(priority=LO)
                else:
                    for cond, nxt in nxts:
                        assert cond is None
                        nxt.lo(ta - cur.ntr, k, sem).start(priority=LO)
                return

            @pl.when(ta < cur.ntr)
            def _():
                cur.lo(ta, k, sem).start(priority=LO)

            for cond, nxt in nxts:
                c = ta >= cur.ntr
                if cond is not None:
                    c = jnp.logical_and(c, cond)

                @pl.when(c)
                def _():
                    nxt.lo(ta - cur.ntr, k, sem).start(priority=LO)

        def stream(cur, hs, nxts, extra=None):
            def body(tr, c):
                for k in range(3):
                    point(cur, tr, k, hs, nxts)
                if extra is not None:
                    extra(tr)
                return c
            lax.fori_loop(0, cur.ntr, body, 0)

        def pro(tr, c):
            for k in range(3):
                wqb_b.lo(tr, k, lsem_at(tr, k)).start(priority=LO)
            return c
        lax.fori_loop(0, DT, pro, 0)
        xb_cp = pltpu.make_async_copy(xb_h, xb_v, xsem.at[0])
        xb_cp.start(priority=HI)
        xa_cp = pltpu.make_async_copy(xa_h, xa_v, xsem.at[1])
        xa_cp.start(priority=HI)

        stream(wqb_b, esem.at[0], [(None, wqa_b)])

        xs[...] = jnp.zeros(xs.shape, F32)
        o_s[...] = jnp.zeros(o_s.shape, F32)
        ctxc_s[...] = jnp.zeros(ctxc_s.shape, F32)
        qa_s[...] = jnp.zeros(qa_s.shape, F32)
        ctx_s[...] = jnp.zeros(ctx_s.shape, F32)
        outb_s[...] = jnp.zeros(outb_s.shape, F32)
        xb_cp.wait()
        xa_cp.wait()
        for s in range(4):
            xs[s, 0:B, :] = xa_v[:, s * 128:(s + 1) * 128].astype(F32)
            xs[4 + s, 0:B, :] = xb_v[:, s * 128:(s + 1) * 128].astype(F32)

        def qb_piece(tr):
            @pl.when(tr == 3)
            def _():
                wqb_b.hi_all(esem.at[0]).wait()

            @pl.when((tr & 3) == 3)
            def _():
                hg = tr >> 2
                x = jnp.concatenate([xs[4 + s] for s in range(4)], axis=-1).astype(BF16)
                w = wqb_v[:, :, pl.ds(pl.multiple_of(hg * 1024, 1024), 1024)].reshape(M, 1024)
                qb_s[hg] = _dot(x, w)

        stream(wqa_b, esem.at[1], [(None, wuk_b)], qb_piece)
        stream(wuk_b, esem.at[2], [(None, ckvb(0))])

        def ckv_body(b, c):
            stream(ckvb(b), esem.at[3 + b], [(b < B - 1, ckvb(jnp.minimum(b + 1, B - 1))), (b == B - 1, wuv_b)])
            return c
        lax.fori_loop(0, B, ckv_body, 0)
        stream(wuv_b, esem.at[7], [(None, wob_b)])
        stream(wob_b, esem.at[8], [(None, kv(0, 0))])

        blk = (lax.broadcasted_iota(jnp.int32, (8, HG * D), 1) >> 7) == lax.broadcasted_iota(jnp.int32, (8, HG * D), 0)

        def tiles(buf, t):
            r = _mo(t * 128, 128)
            return jnp.concatenate([buf[hh, pl.ds(r, 128), :] for hh in range(HG)], axis=-1)

        def qk(ts):
            if not compute:
                return
            qm = qm_s[...].astype(BF16)
            for t in ts:
                s_s[t] = _dot_nt(qm, tiles(kbuf, t))

        def pv(ts):
            if not compute:
                return
            acc = acc_s[...]
            for t in ts:
                acc = acc + _dot(s_s[t].astype(BF16), tiles(vbuf, t))
            acc_s[...] = acc

        def start_k(g):
            if not compute:
                return
            q = qb_s[g >> 2, pl.ds(g & (B - 1), 1), :]
            qm_s[...] = jnp.where(blk, jnp.broadcast_to(q, blk.shape), 0.0)

        def softmax():
            if not compute:
                return
            s = s_s[...]
            m = jnp.max(jnp.max(s, axis=0), axis=-1, keepdims=True)
            p = jnp.exp((s - m[None]) * SCALE)
            l = jnp.sum(jnp.sum(p, axis=0), axis=-1, keepdims=True)
            s_s[...] = p
            l_s[...] = jnp.broadcast_to(l, l_s.shape)
            acc_s[...] = jnp.zeros(acc_s.shape, F32)

        def finish_v(g):
            if not compute:
                return
            o = jnp.where(blk, acc_s[...] / l_s[:, 0:1], 0.0)
            o_s[g >> 2, pl.ds(g & (B - 1), 1), :] = jnp.sum(o, axis=0, keepdims=True)

        def outb_piece(hg):
            outb_s[...] += _dot(o_s[hg].astype(BF16), wob_v[hg])

        def heads(w_v, s):
            return jnp.swapaxes(w_v[s].reshape(128, H, D), 0, 1)

        def a_work_v(g, u):
            @pl.when(g == 0)
            def _():
                @pl.when(u == 0)
                def _():
                    wqa_b.hi_all(esem.at[1]).wait()
                wt = heads(wqa_v, u)
                w = jnp.concatenate([wt[h] for h in range(H)], axis=-1)
                qa_s[...] += _dot(xs[u].astype(BF16), w)

            @pl.when(g == 1)
            def _():
                @pl.when(u == 0)
                def _():
                    wuk_b.hi_all(esem.at[2]).wait()
                wt = heads(wuk_v, u)
                q = qa_s[...].astype(BF16)
                t = jnp.stack([_dot_nt(q[:, h * D:(h + 1) * D], wt[h]) for h in range(H)])
                qabs_s[u] = jnp.swapaxes(t, 0, 1)

            @pl.when(g == 11)
            def _():
                @pl.when(u == 0)
                def _():
                    wuv_b.hi_all(esem.at[7]).wait()
                wt = heads(wuv_v, u)
                c = jnp.swapaxes(ctxc_s[u], 0, 1).astype(BF16)
                ctx_s[...] += jnp.concatenate([_dot(c[h], wt[h]) for h in range(H)], axis=-1)

            @pl.when(jnp.logical_and(g == 13, u < 3))
            def _():
                @pl.when(u == 0)
                def _():
                    wob_b.hi_all(esem.at[8]).wait()
                outb_piece(u)

        def a_work_k(g, u):
            ab = jnp.clip((g - 2) >> 1, 0, B - 1)
            act = jnp.logical_and(g >= 2, g < 10)

            @pl.when(jnp.logical_and(act, (g & 1) == 0))
            def _():
                @pl.when(u == 0)
                def _():
                    ckvb(ab).hi_all(esem.at[3 + ab]).wait()
                q = jnp.concatenate([qabs_s[s, ab] for s in range(4)], axis=-1).astype(BF16)
                sa_s[u] = _dot_nt(q, ckv_v[ab * 4 + u])

            @pl.when(jnp.logical_and(act, (g & 1) == 1))
            def _():
                @pl.when(u == 0)
                def _():
                    s = sa_s[...]
                    m = jnp.max(jnp.max(s, axis=0), axis=-1, keepdims=True)
                    p = jnp.exp((s - m[None]) * SCALE)
                    la_s[...] = jnp.broadcast_to(jnp.sum(jnp.sum(p, axis=0), axis=-1, keepdims=True), la_s.shape)
                    pa_s[...] = p.astype(BF16)
                    acca_s[...] = jnp.zeros(acca_s.shape, F32)
                acca_s[...] += _dot(pa_s[u], ckv_v[ab * 4 + u])

                @pl.when(u == 3)
                def _():
                    c = acca_s[...] / la_s[:, 0:1]
                    for s in range(4):
                        ctxc_s[s, ab] = c[:, s * 128:(s + 1) * 128]

        LT = 20

        def hsem_at(a, j):
            return hsem.at[a * 4 + (j & 3)]

        def phase(a, g):
            cur = kv(a, g)
            if a == 0:
                nxts = [(None, kv(1, g))]
            else:
                nxts = [(g < NG - 1, kv(0, jnp.minimum(g + 1, NG - 1))), (g == NG - 1, woa_b)]
            work = qk if a == 0 else pv

            def group(u, c):
                def pts(lo, hi):
                    for t in range(lo, hi):
                        point(cur, u * 8 + t // 3, t % 3, hsem_at(a, u * 3 + t // 8), nxts)

                def hwait(j):
                    cur.hi_span(j * 128, 128, hsem_at(a, j)).wait()

                pts(0, 8)

                @pl.when(u == 0)
                def _():
                    if a == 0:
                        @pl.when(g > 0)
                        def _():
                            kv(1, g - 1).hi_span(11 * 128, 128, hsem_at(1, 11)).wait()
                            pv([LT + 11])
                            finish_v(g - 1)
                        start_k(g)
                    else:
                        kv(0, g).hi_span(11 * 128, 128, hsem_at(0, 11)).wait()
                        qk([LT + 11])
                        softmax()

                @pl.when(u > 0)
                def _():
                    hwait(u * 3 - 1)
                    work([LT + u * 3 - 1])

                work([u * 5])
                pts(8, 12)
                if acompute:
                    (a_work_k if a == 0 else a_work_v)(g, u)
                pts(12, 16)
                hwait(u * 3)
                work([u * 5 + 1, u * 5 + 2, LT + u * 3])
                pts(16, 24)
                hwait(u * 3 + 1)
                work([u * 5 + 3, u * 5 + 4, LT + u * 3 + 1])
                return c
            lax.fori_loop(0, 4, group, 0)

        def body(g, c):
            phase(0, g)
            phase(1, g)
            return c
        lax.fori_loop(0, NG, body, 0)

        if not acompute:
            wqa_b.hi_all(esem.at[1]).wait()
            wuk_b.hi_all(esem.at[2]).wait()
            for b in range(B):
                ckvb(b).hi_all(esem.at[3 + b]).wait()
            wuv_b.hi_all(esem.at[7]).wait()
            wob_b.hi_all(esem.at[8]).wait()

        def outa(acc, t):
            c = jnp.concatenate([ctx_s[:, s * 1024 + t * 128:s * 1024 + (t + 1) * 128] for s in range(4)], axis=-1)
            w = woa_v[:, t * 128:(t + 1) * 128, :].reshape(512, M)
            r = _dot(c.astype(BF16), w)
            return r if acc is None else acc + r

        def pts(lo, hi):
            for t in range(lo, hi):
                point(woa_b, t // 3, t % 3, hsem_at(0, t // 16), [])

        pts(0, 8)
        kv(1, NG - 1).hi_span(11 * 128, 128, hsem_at(1, 11)).wait()
        pv([LT + 11])
        finish_v(NG - 1)
        pts(8, 12)
        outb_piece(3)
        out_ref[:, M:] = outb_s[0:B, :].astype(out_ref.dtype)
        pts(12, 20)
        acc = outa(None, 0)
        acc = outa(acc, 1)
        pts(20, 30)
        woa_b.hi_span(0, 128, hsem_at(0, 0)).wait()
        acc = outa(acc, 2)
        acc = outa(acc, 5)
        pts(30, 40)
        woa_b.hi_span(128, 128, hsem_at(0, 1)).wait()
        acc = outa(acc, 3)
        acc = outa(acc, 6)
        pts(40, 48)
        acc = outa(acc, 4)
        woa_b.hi_span(256, 128, hsem_at(0, 2)).wait()
        acc = outa(acc, 7)
        out_ref[:, :M] = acc[0:B, :].astype(out_ref.dtype)

    scratch = [
        pltpu.VMEM((HG, SK, D), BF16), pltpu.VMEM((HG, SK, D), BF16),
        pltpu.VMEM((4, 128, H * D), BF16),
        pltpu.VMEM((4, 4096, D), BF16), pltpu.VMEM((4, 4096, D), BF16), pltpu.VMEM((4, 4096, D), BF16),
        pltpu.VMEM((16, 1024, DC), BF16),
        pltpu.VMEM((4, 1024, M), BF16), pltpu.VMEM((4, 1024, M), BF16),
        pltpu.VMEM((B, M), BF16), pltpu.VMEM((B, M), BF16),
        pltpu.VMEM((8, 8, 128), F32),
        pltpu.VMEM((4, 8, HG * D), F32),
        pltpu.VMEM((8, HG * D), F32),
        pltpu.VMEM((32, 8, 128), F32),
        pltpu.VMEM((8, 128), F32),
        pltpu.VMEM((8, HG * D), F32),
        pltpu.VMEM((4, 8, HG * D), F32),
        pltpu.VMEM((8, H * D), F32),
        pltpu.VMEM((4, 8, H, 128), F32),
        pltpu.VMEM((4, H, 1024), F32),
        pltpu.VMEM((4, H, 1024), BF16),
        pltpu.VMEM((H, 128), F32),
        pltpu.VMEM((H, DC), F32),
        pltpu.VMEM((4, 8, H, 128), F32),
        pltpu.VMEM((8, H * D), F32),
        pltpu.VMEM((8, M), F32),
        pltpu.SemaphoreType.DMA((NSEM,)),
        pltpu.SemaphoreType.DMA((8,)),
        pltpu.SemaphoreType.DMA((9,)),
        pltpu.SemaphoreType.DMA((2,)),
    ]

    @jax.jit
    def fn(A_x, A_c_kv, A_w_q, A_w_uk, A_w_uv, A_w_o, B_x, B_k_cache, B_v_cache, B_wq, B_wo):
        out = pl.pallas_call(
            kernel,
            in_specs=[pl.BlockSpec(memory_space=pl.ANY)] * 11,
            out_specs=pl.BlockSpec(memory_space=pltpu.VMEM),
            out_shape=jax.ShapeDtypeStruct((B, 2 * M), BF16),
            scratch_shapes=scratch,
            compiler_params=pltpu.CompilerParams(vmem_limit_bytes=100 * 1024 * 1024, disable_bounds_checks=True),
            name="fused_decode",
        )(A_x.reshape(B, M), A_c_kv.reshape(16, 1024, DC), A_w_q.reshape(4, 4096, D), A_w_uk.reshape(4, 4096, D),
          A_w_uv.reshape(4, 4096, D), A_w_o.reshape(4, 1024, M), B_x.reshape(B, M), B_k_cache, B_v_cache,
          B_wq.reshape(4, 128, H * D), B_wo.reshape(4, 1024, M))
        return out.reshape(B, 1, 2 * M)

    return fn


_fn = make_kernel()


@jax.jit
def pallas_concat_heads__compressed_kv_cla__mha_block_cached__decode_kernel(
    A_x: jax.Array,
    A_c_kv: jax.Array,
    A_w_q: jax.Array,
    A_w_uk: jax.Array,
    A_w_uv: jax.Array,
    A_w_o: jax.Array,
    B_x: jax.Array,
    B_k_cache: jax.Array,
    B_v_cache: jax.Array,
    B_wq: jax.Array,
    B_wo: jax.Array,
):
    return _fn(A_x, A_c_kv, A_w_q, A_w_uk, A_w_uv, A_w_o, B_x, B_k_cache, B_v_cache, B_wq, B_wo)
```

```python
import jax
import jax.numpy as jnp
from jax import lax
import jax.experimental.pallas as pl
import jax.experimental.pallas.tpu as pltpu

B, H, SK, D, M = 4, 32, 4096, 128, 512
DC = 512
HG = 8
NU = B * H
NG = NU // HG
F32 = jnp.float32
BF16 = jnp.bfloat16
LO, HI = 1, 0
SCALE = D ** -0.5


def _dot(a, b):
    return jnp.dot(a, b, preferred_element_type=F32)


def _dot_nt(a, b):
    return lax.dot_general(a, b, (((1,), (1,)), ((), ())), preferred_element_type=F32)


def _mo(x, n):
    return x if isinstance(x, int) else pl.multiple_of(x, n)


class _Block:
    def __init__(self, parts, whole, ntr, lo_idx, hi_idx, hi_rows):
        self.parts, self.whole, self.ntr = parts, whole, ntr
        self.lo_idx, self.hi_idx, self.hi_rows = lo_idx, hi_idx, hi_rows

    def _start(self, idx, sem, prio):
        for src, dst in self.parts:
            pltpu.make_async_copy(src.at[idx], dst.at[idx], sem).start(priority=prio)

    def _wait(self, idx, sem):
        d = self.whole.at[idx]
        pltpu.make_async_copy(d, d, sem).wait()

    def lo_start(self, tr, k, sem):
        self._start(self.lo_idx(tr, k), sem, LO)

    def lo_wait(self, tr, k, sem):
        self._wait(self.lo_idx(tr, k), sem)

    def hi_start(self, tr, k, sem):
        self._start(self.hi_idx(tr, k), sem, HI)

    def hi_wait(self, r, n, sem):
        self._wait((slice(None), pl.ds(_mo(self.hi_rows[0] + r, 8), n)), sem)

    def hi_wait_all(self, sem):
        self.hi_wait(0, self.hi_rows[1], sem)


def _rows_block(parts, whole, pat, hrows, ntr):
    n = len(pat)
    lrows = sum(pat) * ntr

    def lo_idx(tr, k):
        return slice(None), pl.ds(_mo(tr * sum(pat) + sum(pat[:k]), 8), pat[k])

    def hi_idx(tr, k):
        return slice(None), pl.ds(_mo(lrows + (tr * n + k) * hrows, 8), hrows)

    return _Block(parts, whole, ntr, lo_idx, hi_idx, (lrows, hrows * n * ntr))


def _lanes_block(parts, whole, n, ntr, lanes, lw, hpat):
    lper = lanes // lw
    lsh = lper.bit_length() - 1
    lrows = n * ntr // lper * 8
    hsum = sum(hpat)

    def lo_idx(tr, k):
        c = tr * n + k
        return slice(None), pl.ds(_mo((c >> lsh) * 8, 8), 8), pl.ds(_mo((c & (lper - 1)) * lw, 128), lw)

    if hsum <= lanes:
        hper = lanes // hsum
        hsh = hper.bit_length() - 1

        def hi_idx(tr, k):
            return (slice(None), pl.ds(_mo(lrows + (tr >> hsh) * 8, 8), 8),
                    pl.ds(_mo((tr & (hper - 1)) * hsum + sum(hpat[:k]), 128), hpat[k]))
        hrows = ntr // hper * 8
    else:
        g = hsum // lanes

        def hi_idx(tr, k):
            o = sum(hpat[:k])
            return slice(None), pl.ds(_mo(lrows + (tr * g + o // lanes) * 8, 8), 8), pl.ds(o % lanes, hpat[k])
        hrows = ntr * g * 8

    return _Block(parts, whole, ntr, lo_idx, hi_idx, (lrows, hrows))


def make_kernel(mode="53", DT=12, PHI=2, ckv_mode=1, compute=True, acompute=True):
    assert DT < 16
    if mode == "53":
        KV_PAT, P128, P512 = (24, 24, 32), (48, 48, 64), (16, 16, 8)
    else:
        KV_PAT, P128, P512 = (16,) * 4, (32,) * 4, (8,) * 4
    NP = len(KV_PAT)
    GP = 8 * NP
    LTG = 8 * sum(KV_PAT) // 128
    HTG = NP
    LT = 4 * LTG
    HT = 4 * HTG
    assert LT + HT == 32
    ROLL = (HG - PHI) % HG
    CKV_VIEW = {0: (16, 1024, DC), 1: (8, 2048, DC), 2: (8, 2048, DC)}[ckv_mode]

    def kernel(xa_h, ckv_h, wqa_h, wuk_h, wuv_h, woa_h, xb_h, k_h, v_h, wqb_h, wob_h,
               out_ref,
               kbuf, vbuf, wqb_v, wqa_v, wuk_v, wuv_v, ckv_v, woa_v, wob_v, xa_v, xb_v,
               xs, qf_s, q_s, qm_s, s_s, l_s, acc_s, o_s, of_s, ol_s,
               qa_s, qabs_s, sa_s, pa_s, la_s, acca_s, ctxc_s, ctx_s, outb_s,
               lsem, hsem, esem, xsem):

        def n128(src, dst):
            return _rows_block([(src, dst)], dst, P128, 32, 16)

        def n512(src, dst, ntr=16):
            return _rows_block([(src, dst)], dst, P512, 8, ntr)

        def kv(a, g):
            src, dst = (k_h, v_h)[a], (kbuf, vbuf)[a]
            if isinstance(g, int) and g == 0 and ROLL:
                parts = [(src.at[pl.ds(NU - ROLL, ROLL)], dst.at[pl.ds(0, ROLL)]),
                         (src.at[pl.ds(0, HG - ROLL)], dst.at[pl.ds(ROLL, HG - ROLL)])]
            else:
                parts = [(src.at[pl.ds(g * HG - ROLL, HG)], dst)]
            return _rows_block(parts, dst, KV_PAT, 16, 32)

        if ckv_mode == 0:
            NCB = 4

            def ckvb(b):
                return n512(ckv_h.at[pl.ds(b * 4, 4)], ckv_v.at[pl.ds(b * 4, 4)])
        elif ckv_mode == 1:
            NCB = 2

            def ckvb(b):
                return n512(ckv_h.at[pl.ds(b * 4, 4)], ckv_v.at[pl.ds(b * 4, 4)], 32)
        else:
            NCB = 1
            assert mode == "11"

            def ckvb(b):
                return _lanes_block([(ckv_h, ckv_v)], ckv_v, NP, 64, DC, 256, (256,) * 4)

        def ckv_chunk(b, t):
            if ckv_mode == 0:
                return ckv_v[b * 4 + t]
            return ckv_v[b * 2 + (t >> 1), pl.ds(pl.multiple_of((t & 1) * 1024, 1024), 1024), :]

        if mode == "53":
            wqb_b = _lanes_block([(wqb_h, wqb_v)], wqb_v, NP, 16, H * D, 1024, (384, 384, 256))
        else:
            wqb_b = _lanes_block([(wqb_h, wqb_v)], wqb_v, NP, 16, H * D, 512, (512,) * 4)
        wqa_b, wuk_b, wuv_b = n128(wqa_h, wqa_v), n128(wuk_h, wuk_v), n128(wuv_h, wuv_v)
        woa_b, wob_b = n512(woa_h, woa_v), n512(wob_h, wob_v)

        def lsem_at(tr, k):
            return lsem.at[(tr & 15) * NP + k]

        def point(cur, tr, k, hs, nxts):
            if hs is not None:
                cur.hi_start(tr, k, hs)
            cur.lo_wait(tr, k, lsem_at(tr, k))
            ta = tr + DT
            sem = lsem_at(ta, k)
            if isinstance(tr, int):
                if ta < cur.ntr:
                    cur.lo_start(ta, k, sem)
                else:
                    for cond, nxt in nxts:
                        assert cond is None
                        nxt.lo_start(ta - cur.ntr, k, sem)
                return

            @pl.when(ta < cur.ntr)
            def _():
                cur.lo_start(ta, k, sem)

            for cond, nxt in nxts:
                c = ta >= cur.ntr
                if cond is not None:
                    c = jnp.logical_and(c, cond)

                @pl.when(c)
                def _():
                    nxt.lo_start(ta - cur.ntr, k, sem)

        def stream(cur, hs, nxts, extra=None):
            def body(tr, c):
                for k in range(NP):
                    point(cur, tr, k, hs, nxts)
                if extra is not None:
                    extra(tr)
                return c
            lax.fori_loop(0, cur.ntr, body, 0)

        def pro(tr, c):
            for k in range(NP):
                wqb_b.lo_start(tr, k, lsem_at(tr, k))
            return c
        lax.fori_loop(0, DT, pro, 0)
        xb_cp = pltpu.make_async_copy(xb_h, xb_v, xsem.at[0])
        xb_cp.start(priority=HI)
        xa_cp = pltpu.make_async_copy(xa_h, xa_v, xsem.at[1])
        xa_cp.start(priority=HI)

        stream(wqb_b, esem.at[0], [(None, wqa_b)])

        xs[...] = jnp.zeros(xs.shape, F32)
        o_s[...] = jnp.zeros(o_s.shape, F32)
        of_s[...] = jnp.zeros(of_s.shape, F32)
        ctxc_s[...] = jnp.zeros(ctxc_s.shape, F32)
        qa_s[...] = jnp.zeros(qa_s.shape, F32)
        ctx_s[...] = jnp.zeros(ctx_s.shape, F32)
        outb_s[...] = jnp.zeros(outb_s.shape, F32)
        xb_cp.wait()
        xa_cp.wait()
        for s in range(4):
            xs[s, 0:B, :] = xa_v[:, s * 128:(s + 1) * 128].astype(F32)
            xs[4 + s, 0:B, :] = xb_v[:, s * 128:(s + 1) * 128].astype(F32)

        def qb_piece(tr):
            @pl.when(tr == 3)
            def _():
                wqb_b.hi_wait_all(esem.at[0])

            @pl.when((tr & 3) == 3)
            def _():
                hg = tr >> 2
                x = jnp.concatenate([xs[4 + s] for s in range(4)], axis=-1).astype(BF16)
                w = wqb_v[:, :, pl.ds(pl.multiple_of(hg * 1024, 1024), 1024)].reshape(M, 1024)
                q = _dot(x, w)
                q = jnp.swapaxes(jnp.stack([q[:, h * D:(h + 1) * D] for h in range(8)]), 0, 1)
                for b in range(B):
                    qf_s[pl.ds(pl.multiple_of(b * H + hg * 8, 8), 8), :] = q[b]

        stream(wqa_b, esem.at[1], [(None, wuk_b)], qb_piece)
        if ROLL:
            q_s[0:ROLL, :] = qf_s[NU - ROLL:NU, :]
        q_s[ROLL:NU, :] = qf_s[0:NU - ROLL, :]
        stream(wuk_b, esem.at[2], [(None, ckvb(0))])

        if NCB > 1:
            def ckv_body(b, c):
                stream(ckvb(b), esem.at[3], [(b < NCB - 1, ckvb(jnp.minimum(b + 1, NCB - 1))), (b == NCB - 1, wuv_b)])
                return c
            lax.fori_loop(0, NCB, ckv_body, 0)
        else:
            stream(ckvb(0), esem.at[3], [(None, wuv_b)])
        stream(wuv_b, esem.at[4], [(None, wob_b)])
        stream(wob_b, esem.at[5], [(None, kv(0, 0))])

        blk = (lax.broadcasted_iota(jnp.int32, (8, HG * D), 1) >> 7) == lax.broadcasted_iota(jnp.int32, (8, HG * D), 0)

        def tiles(buf, t):
            r = _mo(t * 128, 128)
            return jnp.concatenate([buf[hh, pl.ds(r, 128), :] for hh in range(HG)], axis=-1)

        def qk(ts):
            if not compute or not ts:
                return
            qm = qm_s[...].astype(BF16)
            for t in ts:
                s_s[t] = _dot_nt(qm, tiles(kbuf, t))

        def pv(ts):
            if not compute or not ts:
                return
            acc = acc_s[...]
            for t in ts:
                acc = acc + _dot(s_s[t].astype(BF16), tiles(vbuf, t))
            acc_s[...] = acc

        def start_k(g):
            if not compute:
                return
            q = q_s[pl.ds(_mo(g * HG, HG), HG), :]
            qm_s[...] = jnp.where(blk, jnp.concatenate([q] * HG, axis=-1), 0.0)

        def softmax():
            if not compute:
                return
            s = s_s[...]
            m = jnp.max(jnp.max(s, axis=0), axis=-1, keepdims=True)
            p = jnp.exp((s - m[None]) * SCALE)
            l = jnp.sum(jnp.sum(p, axis=0), axis=-1, keepdims=True)
            s_s[...] = p
            l_s[...] = jnp.broadcast_to(l, l_s.shape)
            acc_s[...] = jnp.zeros(acc_s.shape, F32)

        def finish_v(g):
            if not compute:
                return
            o = jnp.where(blk, acc_s[...], 0.0)
            o8 = o[:, 0:D]
            for hh in range(1, HG):
                o8 = o8 + o[:, hh * D:(hh + 1) * D]
            o_s[pl.ds(_mo(g * HG, HG), HG), :] = o8 / l_s[...]

        def heads(w_v, s):
            return jnp.swapaxes(w_v[s].reshape(128, H, D), 0, 1)

        def a_work_v(g, u):
            @pl.when(g == 1)
            def _():
                @pl.when(u == 0)
                def _():
                    wqa_b.hi_wait_all(esem.at[1])
                wt = heads(wqa_v, u)
                w = jnp.concatenate([wt[h] for h in range(H)], axis=-1)
                qa_s[...] += _dot(xs[u].astype(BF16), w)

            @pl.when(g == 2)
            def _():
                @pl.when(u == 0)
                def _():
                    wuk_b.hi_wait_all(esem.at[2])
                wt = heads(wuk_v, u)
                q = qa_s[...].astype(BF16)
                t = jnp.stack([_dot_nt(q[:, h * D:(h + 1) * D], wt[h]) for h in range(H)])
                qabs_s[u] = jnp.swapaxes(t, 0, 1)

            @pl.when(g == 12)
            def _():
                @pl.when(u == 0)
                def _():
                    wuv_b.hi_wait_all(esem.at[4])
                wt = heads(wuv_v, u)
                c = jnp.swapaxes(ctxc_s[u], 0, 1).astype(BF16)
                ctx_s[...] += jnp.concatenate([_dot(c[h], wt[h]) for h in range(H)], axis=-1)

            @pl.when(g == NG - 1)
            def _():
                @pl.when(u == 0)
                def _():
                    wob_b.hi_wait_all(esem.at[5])
                    if ROLL:
                        of_s[NU - ROLL:NU, :] = o_s[0:ROLL, :]
                    of_s[0:NU - ROLL, :] = o_s[ROLL:NU, :]
                    t = jnp.swapaxes(of_s[...].reshape(8, H, D), 0, 1)
                    for hg in range(4):
                        ol_s[hg] = jnp.concatenate([t[hg * 8 + h] for h in range(8)], axis=-1)
                outb_s[...] += _dot(ol_s[u].astype(BF16), wob_v[u])

        def a_work_k(g, u):
            ab = jnp.clip((g - 3) >> 1, 0, B - 1)
            act = jnp.logical_and(g >= 3, g < 11)

            @pl.when(jnp.logical_and(act, (g & 1) == 1))
            def _():
                @pl.when(jnp.logical_and(g == 3, u == 0))
                def _():
                    for cb in range(NCB):
                        ckvb(cb).hi_wait_all(esem.at[3])
                q = jnp.concatenate([qabs_s[s, ab] for s in range(4)], axis=-1).astype(BF16)
                sa_s[u] = _dot_nt(q, ckv_chunk(ab, u))

            @pl.when(jnp.logical_and(act, (g & 1) == 0))
            def _():
                @pl.when(u == 0)
                def _():
                    s = sa_s[...]
                    m = jnp.max(jnp.max(s, axis=0), axis=-1, keepdims=True)
                    p = jnp.exp((s - m[None]) * SCALE)
                    la_s[...] = jnp.broadcast_to(jnp.sum(jnp.sum(p, axis=0), axis=-1, keepdims=True), la_s.shape)
                    pa_s[...] = p.astype(BF16)
                    acca_s[...] = jnp.zeros(acca_s.shape, F32)
                acca_s[...] += _dot(pa_s[u], ckv_chunk(ab, u))

                @pl.when(u == 3)
                def _():
                    c = acca_s[...] / la_s[:, 0:1]
                    for s in range(4):
                        ctxc_s[s, ab] = c[:, s * 128:(s + 1) * 128]

        def hsem_at(a, j):
            return hsem.at[a * 4 + (j & 3)]

        def ltiles_done(npts):
            rows = (npts // NP) * sum(KV_PAT) + sum(KV_PAT[:npts % NP])
            return rows // 128

        def last_v_tile():
            kv(1, 1).hi_wait((HT - 1) * 128, 128, hsem_at(1, HT - 1))
            pv([LT + HT - 1])

        def phase(a, g):
            first = isinstance(g, int)
            cur = kv(a, g)
            if a == 0:
                nxts = [(None, kv(1, g))]
            elif first:
                nxts = [(None, kv(0, 1))]
            else:
                nxts = [(g < NG - 1, kv(0, jnp.minimum(g + 1, NG - 1))), (g == NG - 1, woa_b)]
            work = qk if a == 0 else pv

            def group(u, c):
                def pts(lo, hi):
                    for t in range(lo, hi):
                        point(cur, u * 8 + t // NP, t % NP, hsem_at(a, u * HTG + t // 8), nxts)

                def hwait(j):
                    cur.hi_wait(j * 128, 128, hsem_at(a, j))

                done = 0
                for i in range(HTG):
                    if i == 1 and acompute and not first:
                        pts(8, 12)
                        (a_work_k if a == 0 else a_work_v)(g, u)
                        pts(12, 16)
                    else:
                        pts(8 * i, 8 * i + 8)
                    now = ltiles_done(8 * i + 8)
                    lts = [u * LTG + t for t in range(done, now)]
                    done = now
                    if i == 0:
                        @pl.when(u == 0)
                        def _():
                            if a == 0:
                                if not first:
                                    last_v_tile()
                                    finish_v(g - 1)
                                start_k(g)
                            else:
                                kv(0, 1).hi_wait((HT - 1) * 128, 128, hsem_at(0, HT - 1))
                                qk([LT + HT - 1])
                                softmax()

                        @pl.when(u > 0)
                        def _():
                            hwait(u * HTG - 1)
                            work([LT + u * HTG - 1])
                        work(lts)
                    else:
                        hwait(u * HTG + i - 1)
                        work(lts + [LT + u * HTG + i - 1])
                return c
            lax.fori_loop(0, 4, group, 0)

        phase(0, 0)
        phase(1, 0)

        def body(g, c):
            phase(0, g)
            phase(1, g)
            return c
        lax.fori_loop(1, NG, body, 0)

        if not acompute:
            wqa_b.hi_wait_all(esem.at[1])
            wuk_b.hi_wait_all(esem.at[2])
            for cb in range(NCB):
                ckvb(cb).hi_wait_all(esem.at[3])
            wuv_b.hi_wait_all(esem.at[4])
            wob_b.hi_wait_all(esem.at[5])

        def outa(acc, t):
            c = jnp.concatenate([ctx_s[:, s * 1024 + t * 128:s * 1024 + (t + 1) * 128] for s in range(4)], axis=-1)
            w = woa_v[:, t * 128:(t + 1) * 128, :].reshape(512, M)
            r = _dot(c.astype(BF16), w)
            return r if acc is None else acc + r

        NPT = 16 * NP
        acc = None
        ldone = 0
        hdone = 0
        for t in range(NPT):
            point(woa_b, t // NP, t % NP, hsem_at(0, t // 16), [])
            if t == 7:
                last_v_tile()
            if t == 11:
                u0 = NU - HG - ROLL
                assert u0 // H == (u0 + HG - 1) // H
                o = jnp.where(blk, acc_s[...] / l_s[:, 0:1], 0.0)
                o = jnp.sum(o, axis=0, keepdims=True)
                rowb = lax.broadcasted_iota(jnp.int32, (8, HG * D), 0) == u0 // H
                o = jnp.where(rowb, jnp.broadcast_to(o, (8, HG * D)), 0.0)
                h0 = u0 % H
                w = jnp.concatenate([wob_v[h // 8, (h % 8) * D:(h % 8 + 1) * D, :] for h in range(h0, h0 + HG)], axis=0)
                out_ref[:, M:] = (outb_s[...] + _dot(o.astype(BF16), w))[0:B, :].astype(out_ref.dtype)
            if t >= 15:
                rows = ((t + 1) // NP) * sum(P512) + sum(P512[:(t + 1) % NP])
                if ldone < rows // 128:
                    acc = outa(acc, ldone)
                    ldone += 1
                elif t + 1 >= 16 * hdone + 16 + 7:
                    woa_b.hi_wait(hdone * 128, 128, hsem_at(0, hdone))
                    acc = outa(acc, LTG + hdone)
                    hdone += 1
        assert ldone == LTG, ldone
        while hdone < HTG:
            woa_b.hi_wait(hdone * 128, 128, hsem_at(0, hdone))
            acc = outa(acc, LTG + hdone)
            hdone += 1
        out_ref[:, :M] = acc[0:B, :].astype(out_ref.dtype)

    scratch = [
        pltpu.VMEM((HG, SK, D), BF16), pltpu.VMEM((HG, SK, D), BF16),
        pltpu.VMEM((4, 128, H * D), BF16),
        pltpu.VMEM((4, 4096, D), BF16), pltpu.VMEM((4, 4096, D), BF16), pltpu.VMEM((4, 4096, D), BF16),
        pltpu.VMEM(CKV_VIEW, BF16),
        pltpu.VMEM((4, 1024, M), BF16), pltpu.VMEM((4, 1024, M), BF16),
        pltpu.VMEM((B, M), BF16), pltpu.VMEM((B, M), BF16),
        pltpu.VMEM((8, 8, 128), F32),
        pltpu.VMEM((NU, D), F32),
        pltpu.VMEM((NU, D), F32),
        pltpu.VMEM((8, HG * D), F32),
        pltpu.VMEM((32, 8, 128), F32),
        pltpu.VMEM((8, 128), F32),
        pltpu.VMEM((8, HG * D), F32),
        pltpu.VMEM((NU, D), F32),
        pltpu.VMEM((8 * H, D), F32),
        pltpu.VMEM((4, 8, HG * D), F32),
        pltpu.VMEM((8, H * D), F32),
        pltpu.VMEM((4, 8, H, 128), F32),
        pltpu.VMEM((4, H, 1024), F32),
        pltpu.VMEM((4, H, 1024), BF16),
        pltpu.VMEM((H, 128), F32),
        pltpu.VMEM((H, DC), F32),
        pltpu.VMEM((4, 8, H, 128), F32),
        pltpu.VMEM((8, H * D), F32),
        pltpu.VMEM((8, M), F32),
        pltpu.SemaphoreType.DMA((16 * NP,)),
        pltpu.SemaphoreType.DMA((8,)),
        pltpu.SemaphoreType.DMA((6,)),
        pltpu.SemaphoreType.DMA((2,)),
    ]

    @jax.jit
    def fn(A_x, A_c_kv, A_w_q, A_w_uk, A_w_uv, A_w_o, B_x, B_k_cache, B_v_cache, B_wq, B_wo):
        out = pl.pallas_call(
            kernel,
            in_specs=[pl.BlockSpec(memory_space=pl.ANY)] * 11,
            out_specs=pl.BlockSpec(memory_space=pltpu.VMEM),
            out_shape=jax.ShapeDtypeStruct((B, 2 * M), BF16),
            scratch_shapes=scratch,
            compiler_params=pltpu.CompilerParams(vmem_limit_bytes=100 * 1024 * 1024, disable_bounds_checks=True),
            name="fused_decode",
        )(A_x.reshape(B, M), A_c_kv.reshape(CKV_VIEW), A_w_q.reshape(4, 4096, D), A_w_uk.reshape(4, 4096, D),
          A_w_uv.reshape(4, 4096, D), A_w_o.reshape(4, 1024, M), B_x.reshape(B, M),
          B_k_cache.reshape(NU, SK, D), B_v_cache.reshape(NU, SK, D),
          B_wq.reshape(4, 128, H * D), B_wo.reshape(4, 1024, M))
        return out.reshape(B, 1, 2 * M)

    return fn


_fn = make_kernel()


@jax.jit
def pallas_concat_heads__compressed_kv_cla__mha_block_cached__decode_kernel(
    A_x: jax.Array,
    A_c_kv: jax.Array,
    A_w_q: jax.Array,
    A_w_uk: jax.Array,
    A_w_uv: jax.Array,
    A_w_o: jax.Array,
    B_x: jax.Array,
    B_k_cache: jax.Array,
    B_v_cache: jax.Array,
    B_wq: jax.Array,
    B_wo: jax.Array,
):
    return _fn(A_x, A_c_kv, A_w_q, A_w_uk, A_w_uv, A_w_o, B_x, B_k_cache, B_v_cache, B_wq, B_wo)
```

```python
import jax
import jax.numpy as jnp
from jax import lax
import jax.experimental.pallas as pl
import jax.experimental.pallas.tpu as pltpu

B, H, SK, D, M = 4, 32, 4096, 128, 512
DC = 512
HG = 8
NU = B * H
NG = NU // HG
F32 = jnp.float32
BF16 = jnp.bfloat16
LO, HI = 1, 0
SCALE = D ** -0.5
NP = 3
HS = 8
ALL = slice(None)


def _dot(a, b):
    return jnp.dot(a, b, preferred_element_type=F32)


def _dot_nt(a, b):
    return lax.dot_general(a, b, (((1,), (1,)), ((), ())), preferred_element_type=F32)


def _mo(x, n):
    return x if isinstance(x, int) else pl.multiple_of(x, n)


class _Rows:
    def __init__(self, src, dst, pat, hrows, ntr, split=True):
        self.src, self.dst, self.pat, self.hrows, self.ntr, self.split = src, dst, pat, hrows, ntr, split
        self.nh = hrows * NP * ntr
        self.h0 = sum(pat) * ntr // 2 if split else sum(pat) * ntr
        self.sh = (ntr // 2).bit_length() - 1

    def lo(self, tr, k):
        r = tr * sum(self.pat) + sum(self.pat[:k])
        if self.split:
            r = r + (tr >> self.sh) * self.nh
        return ALL, pl.ds(_mo(r, 8), self.pat[k])

    def hi(self, j, n=1):
        r = self.h0 + j * self.hrows
        if self.split:
            half = NP * self.ntr // 2
            if isinstance(j, int):
                r = r + (self.nh // 2 if j < half else -self.nh // 2)
            else:
                r = r + jnp.where(j < half, self.nh // 2, -self.nh // 2)
        return ALL, pl.ds(_mo(r, 8), n * self.hrows)

    def hi_all(self):
        return ALL, pl.ds(self.h0, self.nh)


class _Cells:
    ntr = 32

    def __init__(self, src, dst, lg):
        self.src, self.dst, self.lg = src, dst, lg

    def _idx(self, c, off, width):
        return (ALL, pl.ds(_mo((c >> self.lg) * 8, 8), 8),
                pl.ds(_mo((c & ((1 << self.lg) - 1)) * 512 + off, 128), width))

    def lo(self, tr, k):
        c = (tr >> 1) * 5 + (tr >> 4) * 48
        odd = tr & 1
        if k < 2:
            return self._idx(c + k + odd * 3, 0, 512)
        return self._idx(c + 2, odd * 256, 256)

    def hi(self, j):
        hc = j + (128 if j < 48 else 32) if isinstance(j, int) else j + jnp.where(j < 48, 128, 32)
        return self._idx(hc >> 1, (hc & 1) * 256, 256)

    def hi_all(self):
        return ALL, pl.ds((40 >> self.lg) * 8, (48 >> self.lg) * 8)


class _Block:
    def __init__(self, parts, hsem):
        self.parts, self.hsem, self.ntr = parts, hsem, parts[0].ntr

    def _copies(self, f, sem):
        return [pltpu.make_async_copy(p.src.at[f(p)], p.dst.at[f(p)], sem) for p in self.parts]

    def lo_start(self, tr, k, sem):
        for c in self._copies(lambda p: p.lo(tr, k), sem):
            c.start(priority=LO)

    def lo_wait(self, tr, k, sem):
        for c in self._copies(lambda p: p.lo(tr, k), sem):
            c.wait()

    def hi_start(self, j):
        for c in self._copies(lambda p: p.hi(j), self.hsem(j)):
            c.start(priority=HI)

    def hi_wait(self, j, n):
        for c in self._copies(lambda p: p.hi(j, n), self.hsem(j)):
            c.wait()

    def hi_wait_all(self):
        for c in self._copies(lambda p: p.hi_all(), self.hsem(0)):
            c.wait()


def make_kernel(DT=12, DTP=5, compute=True, acompute=True, checks=False, split=True, GSKIP=0,
                SCHED=((3, 'A'), (6, 'L0'), (8, 'H0'), (11, 'L1'), (15, 'L2'), (17, 'H1'), (20, 'L3'), (23, 'H2'), (24, 'L4')),
                TAIL=((42, "aefg"), (46, "bch"), (48, "d"))):
    assert DTP <= DT < 16
    PHI = 2
    KV_PAT, P128, P512 = (24, 24, 32), (48, 48, 64), (16, 16, 8)
    GP = 8 * NP
    ROLL = (HG - PHI) % HG

    def kernel(xa_h, ckv_h, wqa_h, wuk_h, wuv_h, woa_h, xb_h, k_h, v_h, wqb_h, wob_h,
               out_ref,
               kbuf, vbuf, wqb_v, wqa_v, wuk_v, wuv_v, ckv_v, woa_v, wob_v, xa_v, xb_v,
               xs, qf_s, q_s, qm_s, s_s, l_s, acc_s, o_s, of_s, ol_s,
               qa_s, qabs_s, sa_s, pa_s, la_s, acca_s, ctxc_s, ctx_s, outb_s,
               lsem, hsem, esem, xsem, tsem):

        def rows8(src, dst):
            return _Rows(src, dst, KV_PAT, 16, 32, split)

        def kv(a, g):
            src, dst = (k_h, v_h)[a], (kbuf, vbuf)[a]
            return _Block([rows8(src.at[pl.ds(g * HG - ROLL, HG)], dst.at[0])],
                          lambda j: hsem.at[a * 4 + ((j >> 3) & 3)])

        def part(src, dst, u0, n, d0=None):
            d0 = u0 if d0 is None else d0
            s, d = src.at[pl.ds(u0, n)], dst.at[pl.ds(d0, n)]
            lanes = src.shape[-1]
            return rows8(s, d) if lanes == 128 else _Cells(s, d, 0 if lanes == 512 else 3)

        k0, v0 = kbuf.at[1], vbuf.at[1]
        pre = [
            [part(wob_h, wob_v, 2, 2), part(wqb_h, wqb_v, 0, 4), part(v_h, v0, 0, PHI, ROLL)],
            [part(wuk_h, wuk_v, 2, 2), part(wqa_h, wqa_v, 0, 4), part(ckv_h, ckv_v, 0, 2)],
            [part(wuv_h, wuv_v, 0, 4), part(wuk_h, wuk_v, 0, 2)],
            [part(ckv_h, ckv_v, 2, 8)],
            [part(ckv_h, ckv_v, 10, 6)],
            [part(k_h, k0, NU - ROLL, ROLL, 0), part(wob_h, wob_v, 0, 2)],
            [part(v_h, v0, NU - ROLL, ROLL, 0), part(k_h, k0, 0, PHI, ROLL)],
        ]
        pre = [_Block(p, lambda j, i=i: esem.at[i & 1]) for i, p in enumerate(pre)]

        def woa_sem(j):
            assert isinstance(j, int)
            return tsem.at[j // 16] if j < 32 else tsem.at[2 + (j - 32) // 4]
        woa_b = _Block([_Rows(woa_h, woa_v, P512, 8, 16, False)], woa_sem)

        def lsem_at(tr, k):
            return lsem.at[(tr & 15) * NP + k]

        def either(pos, lim, cur_fn, nxts, nxt_fn):
            if isinstance(pos, int):
                if pos < lim:
                    cur_fn()
                else:
                    for cond, nxt in nxts:
                        assert cond is None
                        nxt_fn(nxt)
                return
            pl.when(pos < lim)(cur_fn)
            for cond, nxt in nxts:
                c = pos >= lim
                if cond is not None:
                    c = jnp.logical_and(c, cond)
                pl.when(c)(lambda nxt=nxt: nxt_fn(nxt))

        def point(cur, tr, k, nxts, dt, h_in_cur=False, h_next=None):
            j = tr * NP + k + HS
            nj = NP * cur.ntr
            if h_in_cur:
                cur.hi_start(j)
            else:
                either(j, nj, lambda: cur.hi_start(j), nxts,
                       lambda nxt: nxt.hi_start(j - nj if h_next is None else h_next))
            cur.lo_wait(tr, k, lsem_at(tr, k))
            ta = tr + dt
            sem = lsem_at(ta, k)
            either(ta, cur.ntr, lambda: cur.lo_start(ta, k, sem), nxts,
                   lambda nxt: nxt.lo_start(ta - cur.ntr, k, sem))

        def stream(cur, nxt, extra=None):
            def body(tr, c):
                for k in range(NP):
                    point(cur, tr, k, [(None, nxt)], DTP)
                if extra is not None:
                    extra(tr)
                return c
            lax.fori_loop(0, cur.ntr, body, 0)

        def pro(tr, c):
            @pl.when(tr < DTP)
            def _():
                for k in range(NP):
                    pre[0].lo_start(tr, k, lsem_at(tr, k))
            pre[0].hi_start(tr)
            return c
        lax.fori_loop(0, HS, pro, 0)
        assert DTP <= HS
        xb_cp = pltpu.make_async_copy(xb_h, xb_v, xsem.at[0])
        xb_cp.start(priority=HI)
        xa_cp = pltpu.make_async_copy(xa_h, xa_v, xsem.at[1])
        xa_cp.start(priority=HI)

        stream(pre[0], pre[1])

        xs[...] = jnp.zeros(xs.shape, F32)
        o_s[...] = jnp.zeros(o_s.shape, F32)
        of_s[...] = jnp.zeros(of_s.shape, F32)
        ctxc_s[...] = jnp.zeros(ctxc_s.shape, F32)
        qa_s[...] = jnp.zeros(qa_s.shape, F32)
        ctx_s[...] = jnp.zeros(ctx_s.shape, F32)
        outb_s[...] = jnp.zeros(outb_s.shape, F32)
        xb_cp.wait()
        xa_cp.wait()
        for s in range(4):
            xs[s, 0:B, :] = xa_v[:, s * 128:(s + 1) * 128].astype(F32)
            xs[4 + s, 0:B, :] = xb_v[:, s * 128:(s + 1) * 128].astype(F32)
        pre[0].hi_wait_all()

        def qb_piece(tr):
            @pl.when(jnp.logical_and((tr & 3) == 3, tr < 16))
            def _():
                hg = tr >> 2
                x = jnp.concatenate([xs[4 + s] for s in range(4)], axis=-1).astype(BF16)
                w = wqb_v[:, :, pl.ds(pl.multiple_of(hg * 1024, 1024), 1024)].reshape(M, 1024)
                q = _dot(x, w)
                q = jnp.swapaxes(jnp.stack([q[:, h * D:(h + 1) * D] for h in range(8)]), 0, 1)
                for b in range(B):
                    qf_s[pl.ds(pl.multiple_of(b * H + hg * 8, 8), 8), :] = q[b]

        for i in range(1, len(pre)):
            stream(pre[i], pre[i + 1] if i + 1 < len(pre) else kv(0, 1 + GSKIP), qb_piece if i == 1 else None)
            pre[i].hi_wait_all()
            if i == 1:
                if ROLL:
                    q_s[0:ROLL, :] = qf_s[NU - ROLL:NU, :]
                q_s[ROLL:NU, :] = qf_s[0:NU - ROLL, :]

        def deepen(tr, c):
            for k in range(NP):
                kv(0, 1 + GSKIP).lo_start(tr, k, lsem_at(tr, k))
            return c
        lax.fori_loop(DTP, DT, deepen, 0)

        blk = (lax.broadcasted_iota(jnp.int32, (8, HG * D), 1) >> 7) == lax.broadcasted_iota(jnp.int32, (8, HG * D), 0)

        def tiles(buf, z, t):
            r = _mo(t * 128, 128)
            return jnp.concatenate([buf[z, hh, pl.ds(r, 128), :] for hh in range(HG)], axis=-1)

        def qk(ts, z=0):
            if not compute or not ts:
                return
            qm = qm_s[z].astype(BF16)
            for t in ts:
                s_s[z, t] = _dot_nt(qm, tiles(kbuf, z, t))

        def pv(ts, z=0):
            if not compute or not ts:
                return
            acc = acc_s[z]
            for t in ts:
                acc = acc + _dot(s_s[z, t].astype(BF16), tiles(vbuf, z, t))
            acc_s[z] = acc

        def start_k(g, z=0):
            if not compute:
                return
            q = q_s[pl.ds(_mo(g * HG, HG), HG), :]
            qm_s[z] = jnp.where(blk, jnp.concatenate([q] * HG, axis=-1), 0.0)

        def softmax(z=0):
            if not compute:
                return
            s = s_s[z]
            m = jnp.max(jnp.max(s, axis=0), axis=-1, keepdims=True)
            p = jnp.exp((s - m[None]) * SCALE)
            l = jnp.sum(jnp.sum(p, axis=0), axis=-1, keepdims=True)
            s_s[z] = p
            l_s[z] = jnp.broadcast_to(l, (8, 128))
            acc_s[z] = jnp.zeros((8, HG * D), F32)

        def finish_v(g, z=0):
            if not compute:
                return
            o = jnp.where(blk, acc_s[z], 0.0)
            o8 = o[:, 0:D]
            for hh in range(1, HG):
                o8 = o8 + o[:, hh * D:(hh + 1) * D]
            o_s[pl.ds(_mo(g * HG, HG), HG), :] = o8 / l_s[z]

        start_k(0, 1)

        def heads(w_v, s):
            return jnp.swapaxes(w_v[s].reshape(128, H, D), 0, 1)

        def a_work_v(g, u):
            @pl.when(g == 1)
            def _():
                wt = heads(wqa_v, u)
                w = jnp.concatenate([wt[h] for h in range(H)], axis=-1)
                qa_s[...] += _dot(xs[u].astype(BF16), w)

            @pl.when(g == 2)
            def _():
                wt = heads(wuk_v, u)
                q = qa_s[...].astype(BF16)
                t = jnp.stack([_dot_nt(q[:, h * D:(h + 1) * D], wt[h]) for h in range(H)])
                qabs_s[u] = jnp.swapaxes(t, 0, 1)

            t0 = (((g - 3) & 3) * 4 + u) * 2

            @pl.when(jnp.logical_and(g >= 3, g < 7))
            def _():
                qk([t0, t0 + 1], 1)

                @pl.when(t0 == 30)
                def _():
                    softmax(1)

            @pl.when(jnp.logical_and(g >= 7, g < 11))
            def _():
                pv([t0, t0 + 1], 1)

                @pl.when(t0 == 30)
                def _():
                    finish_v(0, 1)

            @pl.when(g == 12)
            def _():
                wt = heads(wuv_v, u)
                c = jnp.swapaxes(ctxc_s[u], 0, 1).astype(BF16)
                ctx_s[...] += jnp.concatenate([_dot(c[h], wt[h]) for h in range(H)], axis=-1)

            @pl.when(g == NG - 1)
            def _():
                @pl.when(u == 0)
                def _():
                    if ROLL:
                        of_s[NU - ROLL:NU, :] = o_s[0:ROLL, :]
                    of_s[0:NU - ROLL, :] = o_s[ROLL:NU, :]
                    t = jnp.swapaxes(of_s[...].reshape(8, H, D), 0, 1)
                    for hg in range(4):
                        ol_s[hg] = jnp.concatenate([t[hg * 8 + h] for h in range(8)], axis=-1)
                outb_s[...] += _dot(ol_s[u].astype(BF16), wob_v[u])

        def a_work_k(g, u):
            ab = jnp.clip((g - 3) >> 1, 0, B - 1)
            act = jnp.logical_and(g >= 3, g < 11)

            @pl.when(jnp.logical_and(act, (g & 1) == 1))
            def _():
                q = jnp.concatenate([qabs_s[s, ab] for s in range(4)], axis=-1).astype(BF16)
                sa_s[u] = _dot_nt(q, ckv_v[ab * 4 + u])

            @pl.when(jnp.logical_and(act, (g & 1) == 0))
            def _():
                @pl.when(u == 0)
                def _():
                    s = sa_s[...]
                    m = jnp.max(jnp.max(s, axis=0), axis=-1, keepdims=True)
                    p = jnp.exp((s - m[None]) * SCALE)
                    la_s[...] = jnp.broadcast_to(jnp.sum(jnp.sum(p, axis=0), axis=-1, keepdims=True), la_s.shape)
                    pa_s[...] = p.astype(BF16)
                    acca_s[...] = jnp.zeros(acca_s.shape, F32)
                acca_s[...] += _dot(pa_s[u], ckv_v[ab * 4 + u])

                @pl.when(u == 3)
                def _():
                    c = acca_s[...] / la_s[:, 0:1]
                    for s in range(4):
                        ctxc_s[s, ab] = c[:, s * 128:(s + 1) * 128]

        def ltiles_done(npts):
            rows = (npts // NP) * sum(KV_PAT) + sum(KV_PAT[:npts % NP])
            return rows // 128

        def phase(a, g):
            cur = kv(a, g)
            if a == 0:
                nxts = [(None, kv(1, g))]
            else:
                nxts = [(g < NG - 1, kv(0, jnp.minimum(g + 1, NG - 1))), (g == NG - 1, woa_b)]
            work = qk if a == 0 else pv
            if a == 0:
                start_k(g)

            def group(u, c):
                for t in range(GP):
                    point(cur, u * 8 + t // NP, t % NP, nxts, DT, h_in_cur=t + HS < GP, h_next=t + HS - GP)
                    for tt, items in SCHED:
                        if tt != t + 1:
                            continue
                        ts = []
                        for item in items.split("+"):
                            if item == "A":
                                if acompute:
                                    (a_work_k if a == 0 else a_work_v)(g, u)
                            elif item[0] == "L":
                                j = int(item[1])
                                assert j < ltiles_done(t + 1)
                                ts.append(u * 5 + j + (u >> 1) * 12 if split else u * 5 + j)
                            else:
                                j = int(item[1])
                                assert t + 1 >= 8 * j
                                cur.hi_wait((u * 3 + j) * 8, 8)
                                ts.append(16 + u * 3 + j - (u >> 1) * 12 if split else 20 + u * 3 + j)
                        work(ts)
                return c
            lax.fori_loop(0, 4, group, 0)
            if a == 0:
                softmax()
            else:
                finish_v(g)

        def body(g, c):
            phase(0, g)
            phase(1, g)
            return c
        lax.fori_loop(1 + GSKIP, NG, body, 0)

        def outa(acc, t):
            c = jnp.concatenate([ctx_s[:, s * 1024 + t * 128:s * 1024 + (t + 1) * 128] for s in range(4)], axis=-1)
            w = woa_v[:, t * 128:(t + 1) * 128, :].reshape(512, M)
            r = _dot(c.astype(BF16), w)
            return r if acc is None else acc + r

        qrow = {n: 512 + 32 * i for i, n in enumerate("abcd")}
        qrow.update({n: 896 + 32 * i for i, n in enumerate("efgh")})

        acc = None
        lhs = {}
        for t in range(16 * NP):
            point(woa_b, t // NP, t % NP, [], DT)
            if t + 1 == 3:
                u0 = NU - HG - ROLL
                assert u0 // H == (u0 + HG - 1) // H
                o = jnp.where(blk, acc_s[0] / l_s[0][:, 0:1], 0.0)
                o = jnp.sum(o, axis=0, keepdims=True)
                rowb = lax.broadcasted_iota(jnp.int32, (8, HG * D), 0) == u0 // H
                o = jnp.where(rowb, jnp.broadcast_to(o, (8, HG * D)), 0.0)
                h0 = u0 % H
                w = jnp.concatenate([wob_v[h // 8, (h % 8) * D:(h % 8 + 1) * D, :] for h in range(h0, h0 + HG)], axis=0)
                out_ref[:, M:] = (outb_s[...] + _dot(o.astype(BF16), w))[0:B, :].astype(out_ref.dtype)
            if t + 1 == 11:
                acc = outa(acc, 0)
            if t + 1 == 15:
                woa_b.hi_wait(0, 16)
                acc = outa(acc, 5)
            if t + 1 == 20:
                acc = outa(acc, 1)
            if t + 1 == 24:
                for _, names in TAIL:
                    lhs[names] = jnp.concatenate(
                        [ctx_s[:, s * 1024 + qrow[n]:s * 1024 + qrow[n] + 32] for n in names for s in range(4)],
                        axis=-1).astype(BF16)
            if t + 1 == 29:
                acc = outa(acc, 2)
            if t + 1 == 33:
                woa_b.hi_wait(16, 16)
                acc = outa(acc, 6)
            if t + 1 == 38:
                acc = outa(acc, 3)
            for tt, names in TAIL:
                if tt == t + 1:
                    rows = ((t + 1) // NP) * sum(P512) + sum(P512[:(t + 1) % NP])
                    for n in names:
                        if n in "abcd":
                            assert qrow[n] + 32 <= rows
                        else:
                            woa_b.hi_wait(32 + 4 * "efgh".index(n), 4)
                    w = jnp.concatenate([woa_v[s, qrow[n]:qrow[n] + 32, :] for n in names for s in range(4)], axis=0)
                    acc = acc + _dot(lhs[names], w)
        out_ref[:, :M] = acc[0:B, :].astype(out_ref.dtype)

    scratch = [
        pltpu.VMEM((2, HG, SK, D), BF16), pltpu.VMEM((2, HG, SK, D), BF16),
        pltpu.VMEM((4, 128, H * D), BF16),
        pltpu.VMEM((4, 4096, D), BF16), pltpu.VMEM((4, 4096, D), BF16), pltpu.VMEM((4, 4096, D), BF16),
        pltpu.VMEM((16, 1024, DC), BF16),
        pltpu.VMEM((4, 1024, M), BF16), pltpu.VMEM((4, 1024, M), BF16),
        pltpu.VMEM((B, M), BF16), pltpu.VMEM((B, M), BF16),
        pltpu.VMEM((8, 8, 128), F32),
        pltpu.VMEM((NU, D), F32),
        pltpu.VMEM((NU, D), F32),
        pltpu.VMEM((2, 8, HG * D), F32),
        pltpu.VMEM((2, 32, 8, 128), F32),
        pltpu.VMEM((2, 8, 128), F32),
        pltpu.VMEM((2, 8, HG * D), F32),
        pltpu.VMEM((NU, D), F32),
        pltpu.VMEM((8 * H, D), F32),
        pltpu.VMEM((4, 8, HG * D), F32),
        pltpu.VMEM((8, H * D), F32),
        pltpu.VMEM((4, 8, H, 128), F32),
        pltpu.VMEM((4, H, 1024), F32),
        pltpu.VMEM((4, H, 1024), BF16),
        pltpu.VMEM((H, 128), F32),
        pltpu.VMEM((H, DC), F32),
        pltpu.VMEM((4, 8, H, 128), F32),
        pltpu.VMEM((8, H * D), F32),
        pltpu.VMEM((8, M), F32),
        pltpu.SemaphoreType.DMA((16 * NP,)),
        pltpu.SemaphoreType.DMA((8,)),
        pltpu.SemaphoreType.DMA((2,)),
        pltpu.SemaphoreType.DMA((2,)),
        pltpu.SemaphoreType.DMA((6,)),
    ]

    @jax.jit
    def fn(A_x, A_c_kv, A_w_q, A_w_uk, A_w_uv, A_w_o, B_x, B_k_cache, B_v_cache, B_wq, B_wo):
        out = pl.pallas_call(
            kernel,
            in_specs=[pl.BlockSpec(memory_space=pl.ANY)] * 11,
            out_specs=pl.BlockSpec(memory_space=pltpu.VMEM),
            out_shape=jax.ShapeDtypeStruct((B, 2 * M), BF16),
            scratch_shapes=scratch,
            compiler_params=pltpu.CompilerParams(vmem_limit_bytes=100 * 1024 * 1024, disable_bounds_checks=not checks,
                                                 disable_semaphore_checks=not checks),
            name="fused_decode",
        )(A_x.reshape(B, M), A_c_kv.reshape(16, 1024, DC), A_w_q.reshape(4, 4096, D), A_w_uk.reshape(4, 4096, D),
          A_w_uv.reshape(4, 4096, D), A_w_o.reshape(4, 1024, M), B_x.reshape(B, M),
          B_k_cache.reshape(NU, SK, D), B_v_cache.reshape(NU, SK, D),
          B_wq.reshape(4, 128, H * D), B_wo.reshape(4, 1024, M))
        return out.reshape(B, 1, 2 * M)

    return fn


_fn = make_kernel()


@jax.jit
def pallas_concat_heads__compressed_kv_cla__mha_block_cached__decode_kernel(
    A_x: jax.Array,
    A_c_kv: jax.Array,
    A_w_q: jax.Array,
    A_w_uk: jax.Array,
    A_w_uv: jax.Array,
    A_w_o: jax.Array,
    B_x: jax.Array,
    B_k_cache: jax.Array,
    B_v_cache: jax.Array,
    B_wq: jax.Array,
    B_wo: jax.Array,
):
    return _fn(A_x, A_c_kv, A_w_q, A_w_uk, A_w_uv, A_w_o, B_x, B_k_cache, B_v_cache, B_wq, B_wo)
```

```python
import jax
import jax.numpy as jnp
from jax import lax
import jax.experimental.pallas as pl
import jax.experimental.pallas.tpu as pltpu

B, H, SK, D, M = 4, 32, 4096, 128, 512
DC = 512
HG = 8
NU = B * H
NG = NU // HG
F32 = jnp.float32
BF16 = jnp.bfloat16
LO, HI = 1, 0
SCALE = D ** -0.5
NP = 3
HS = 8
PHI = 2
ROLL = HG - PHI
ALL = slice(None)


def _dot(a, b):
    return jnp.dot(a, b, preferred_element_type=F32)


def _dot_nt(a, b):
    return lax.dot_general(a, b, (((1,), (1,)), ((), ())), preferred_element_type=F32)


def _mo(x, n):
    return x if isinstance(x, int) else pl.multiple_of(x, n)


def _sel(c, a, b):
    return (a if c else b) if isinstance(c, bool) else jnp.where(c, a, b)


class _Rows:
    ntr = 32
    pat = (24, 24, 32)
    UP_UP = ((0, 1), (2816, 1), (2048, 1), (1280, 1))
    UP_DOWN = ((0, 1), (3328, -1), (4096, -1), (1280, 1))

    def __init__(self, src, dst, walk):
        self.src, self.dst, self.walk = src, dst, walk

    def _row(self, first, seg, off, half, n):
        def pos(s, o):
            return s[0] + o if s[1] > 0 else s[0] - o - n
        return _sel(first, pos(self.walk[seg], off), pos(self.walk[seg + 1], off - half))

    def lo(self, tr, k):
        r = self._row(tr < 16, 0, tr * 80 + sum(self.pat[:k]), 1280, self.pat[k])
        return ALL, pl.ds(_mo(r, 8), self.pat[k])

    def hi(self, j, n=1):
        return ALL, pl.ds(_mo(self._row(j < 48, 2, j * 16, 768, n * 16), 8), n * 16)

    def hi_all(self):
        assert self.walk == self.UP_UP
        return ALL, pl.ds(1280, 1536)

    def lo_tile(self, u, i):
        return self._row(u < 2, 0, (u * 5 + i) * 128, 1280, 128)

    def hi_tile(self, u, i):
        return self._row(u < 2, 2, (u * 3 + i) * 128, 768, 128)


class _Cells:
    ntr = 32

    def __init__(self, src, dst, lg):
        self.src, self.dst, self.lg = src, dst, lg

    def _idx(self, c, off, width):
        return (ALL, pl.ds(_mo((c >> self.lg) * 8, 8), 8),
                pl.ds(_mo((c & ((1 << self.lg) - 1)) * 512 + off, 128), width))

    def lo(self, tr, k):
        c = (tr >> 1) * 5 + (tr >> 4) * 48
        odd = tr & 1
        if k < 2:
            return self._idx(c + k + odd * 3, 0, 512)
        return self._idx(c + 2, odd * 256, 256)

    def hi(self, j):
        hc = j + _sel(j < 48, 128, 32)
        return self._idx(hc >> 1, (hc & 1) * 256, 256)

    def hi_all(self):
        return ALL, pl.ds((40 >> self.lg) * 8, (48 >> self.lg) * 8)


class _Last:
    ntr = 16
    pat = (16, 16, 8)

    def __init__(self, src, dst):
        self.src, self.dst = src, dst

    def lo(self, tr, k):
        return ALL, pl.ds(_mo(tr * 40 + sum(self.pat[:k]), 8), self.pat[k])

    def hi(self, j, n=1):
        return ALL, pl.ds(640 + j * 8, n * 8)


class _Block:
    def __init__(self, parts, hsem):
        self.parts, self.hsem, self.ntr = parts, hsem, parts[0].ntr

    def _copies(self, idx, sem):
        return [pltpu.make_async_copy(p.src.at[idx(p)], p.dst.at[idx(p)], sem(i)) for i, p in enumerate(self.parts)]

    def lo_start(self, tr, k, sem):
        for c in self._copies(lambda p: p.lo(tr, k), lambda i: sem):
            c.start(priority=LO)

    def lo_wait(self, tr, k, sem):
        for c in self._copies(lambda p: p.lo(tr, k), lambda i: sem):
            c.wait()

    def hi_start(self, j):
        for c in self._copies(lambda p: p.hi(j), lambda i: self.hsem(j, i)):
            c.start(priority=HI)

    def hi_wait(self, j, n):
        for c in self._copies(lambda p: p.hi(j, n), lambda i: self.hsem(j, i)):
            c.wait()

    def hi_wait_all(self):
        for c in self._copies(lambda p: p.hi_all(), lambda i: self.hsem(0, i)):
            c.wait()


def make_kernel(DT=12, DTP=5, checks=False,
                SCHED=((3, "A0"), (6, "L0"), (8, "H0"), (11, "L1"), (13, "A1"), (16, "L2"), (18, "H1"), (20, "L3"),
                       (23, "H2"), (24, "L4")),
                TAIL=((39, "ef"), (44, "abg"), (48, "cdh"))):
    assert DTP <= DT < 16
    NQ = 2
    HQ = H // NQ
    CQ = 1024 // NQ
    GP = 8 * NP

    def kernel(xa_h, ckv_h, wqa_h, wuk_h, wuv_h, woa_h, xb_h, k_h, v_h, wqb_h, wob_h,
               out_ref,
               kbuf, vbuf, wqb_v, wqa_v, wuk_v, wuv_v, ckv_v, woa_v, wob_v, xa_v, xb_v,
               xs, qf_s, q_s, qm_s, s_s, l_s, acc_s, o_s, of_s, ol_s,
               qa_s, qabs_s, sa_s, ma_s, la_s, acca_s, ctxc_s, ctx_s, outb_s,
               lsem, hsem, esem, xsem, tsem):

        def kv(a, g):
            src, dst = (k_h, v_h)[a], (kbuf, vbuf)[a]
            return _Block([_Rows(src.at[pl.ds(g * HG - ROLL, HG)], dst.at[0], _Rows.UP_DOWN)],
                          lambda j, i: hsem.at[a * 4 + ((j >> 3) & 3)])

        def part(src, dst, u0, n, d0=None):
            s, d = src.at[pl.ds(u0, n)], dst.at[pl.ds(u0 if d0 is None else d0, n)]
            lanes = src.shape[-1]
            return _Rows(s, d, _Rows.UP_UP) if lanes == 128 else _Cells(s, d, 0 if lanes == 512 else 3)

        k0, v0 = kbuf.at[1], vbuf.at[1]
        pre = [
            [part(wob_h, wob_v, 2, 2), part(wqb_h, wqb_v, 0, 4), part(v_h, v0, 0, PHI, ROLL)],
            [part(wuk_h, wuk_v, 2, 2), part(wqa_h, wqa_v, 0, 4), part(ckv_h, ckv_v, 0, 2)],
            [part(wuv_h, wuv_v, 0, 4), part(wuk_h, wuk_v, 0, 2)],
            [part(ckv_h, ckv_v, 2, 8)],
            [part(ckv_h, ckv_v, 10, 6)],
            [part(k_h, k0, NU - ROLL, ROLL, 0), part(wob_h, wob_v, 0, 2)],
            [part(v_h, v0, NU - ROLL, ROLL, 0), part(k_h, k0, 0, PHI, ROLL)],
        ]
        pre = [_Block(p, lambda j, i, n=n: esem.at[(n & 1) * 3 + i]) for n, p in enumerate(pre)]
        last = _Block([_Last(woa_h, woa_v)], lambda j, i: tsem.at[j // 16 if j < 32 else 2 + (j - 32) // 4])

        def lsem_at(tr, k):
            return lsem.at[(tr & 15) * NP + k]

        def either(pos, lim, cur_fn, nxts, nxt_fn):
            if isinstance(pos, int):
                if pos < lim:
                    cur_fn()
                else:
                    assert not nxts
                return
            pl.when(pos < lim)(cur_fn)
            for cond, nxt in nxts:
                c = pos >= lim
                if cond is not None:
                    c = jnp.logical_and(c, cond)
                pl.when(c)(lambda nxt=nxt: nxt_fn(nxt))

        def point(cur, tr, k, nxts, dt, h_in_cur=False, h_next=None):
            j = tr * NP + k + HS
            nj = NP * cur.ntr
            if h_in_cur:
                cur.hi_start(j)
            else:
                either(j, nj, lambda: cur.hi_start(j), nxts,
                       lambda nxt: nxt.hi_start(j - nj if h_next is None else h_next))
            cur.lo_wait(tr, k, lsem_at(tr, k))
            ta = tr + dt
            sem = lsem_at(ta, k)
            either(ta, cur.ntr, lambda: cur.lo_start(ta, k, sem), nxts,
                   lambda nxt: nxt.lo_start(ta - cur.ntr, k, sem))

        def stream(cur, nxt, extra=None):
            def body(tr, c):
                for k in range(NP):
                    point(cur, tr, k, [(None, nxt)], DTP)
                if extra is not None:
                    extra(tr)
                return c
            lax.fori_loop(0, cur.ntr, body, 0)
            cur.hi_wait_all()

        zeroed = [[xs, o_s, qa_s], [of_s, ctx_s, outb_s, ma_s], [ctxc_s.at[0], ctxc_s.at[1]], [ctxc_s.at[2], ctxc_s.at[3]]]
        xb_cp = pltpu.make_async_copy(xb_h, xb_v, xsem.at[0])
        xa_cp = pltpu.make_async_copy(xa_h, xa_v, xsem.at[1])
        for j in range(HS):
            if j < DTP:
                for k in range(NP):
                    pre[0].lo_start(j, k, lsem_at(j, k))
            pre[0].hi_start(j)
            if j == 2:
                xb_cp.start(priority=HI)
                xa_cp.start(priority=HI)
            if j >= HS - len(zeroed):
                for r in zeroed[j - HS]:
                    r[...] = jnp.zeros(r.shape, F32)
        assert DTP <= HS

        stream(pre[0], pre[1])

        xb_cp.wait()
        xa_cp.wait()
        for s in range(4):
            xs[s, 0:B, :] = xa_v[:, s * 128:(s + 1) * 128].astype(F32)
            xs[4 + s, 0:B, :] = xb_v[:, s * 128:(s + 1) * 128].astype(F32)

        def qb_piece(tr):
            @pl.when((tr & 7) == 3)
            def _():
                hg = tr >> 3
                x = jnp.concatenate([xs[4 + s] for s in range(4)], axis=-1).astype(BF16)
                w = wqb_v[:, :, pl.ds(pl.multiple_of(hg * 1024, 1024), 1024)].reshape(M, 1024)
                q = _dot(x, w)
                q = jnp.swapaxes(jnp.stack([q[:, h * D:(h + 1) * D] for h in range(8)]), 0, 1)
                for b in range(B):
                    qf_s[pl.ds(pl.multiple_of(b * H + hg * 8, 8), 8), :] = q[b]

        stream(pre[1], pre[2], qb_piece)
        q_s[0:ROLL, :] = qf_s[NU - ROLL:NU, :]
        q_s[ROLL:NU, :] = qf_s[0:NU - ROLL, :]
        for n in range(2, len(pre)):
            stream(pre[n], pre[n + 1] if n + 1 < len(pre) else kv(0, 1))

        def deepen(tr, c):
            for k in range(NP):
                kv(0, 1).lo_start(tr, k, lsem_at(tr, k))
            return c
        lax.fori_loop(DTP, DT, deepen, 0)

        blk = (lax.broadcasted_iota(jnp.int32, (8, HG * D), 1) >> 7) == lax.broadcasted_iota(jnp.int32, (8, HG * D), 0)

        def tile(buf, z, r):
            r = pl.multiple_of(r, 128)
            return jnp.concatenate([buf[z, i, pl.ds(r, 128), :] for i in range(HG)], axis=-1)

        def qk(r, z=0):
            s_s[z, r >> 7] = _dot_nt(qm_s[z].astype(BF16), tile(kbuf, z, r))

        def pv(r, z=0):
            acc_s[z] += _dot(s_s[z, r >> 7].astype(BF16), tile(vbuf, z, r))

        def start_k(g, z=0):
            q = q_s[pl.ds(_mo(g * HG, HG), HG), :]
            qm_s[z] = jnp.where(blk, jnp.concatenate([q] * HG, axis=-1), 0.0)

        def softmax(z=0):
            s = s_s[z]
            m = jnp.max(jnp.max(s, axis=0), axis=-1, keepdims=True)
            p = jnp.exp((s - m[None]) * SCALE)
            l = jnp.sum(jnp.sum(p, axis=0), axis=-1, keepdims=True)
            s_s[z] = p
            l_s[z] = jnp.broadcast_to(l, (8, 128))
            acc_s[z] = jnp.zeros((8, HG * D), F32)

        def finish_v(g, z=0):
            o = jnp.where(blk, acc_s[z], 0.0)
            o8 = o[:, 0:D]
            for i in range(1, HG):
                o8 = o8 + o[:, i * D:(i + 1) * D]
            o_s[pl.ds(_mo(g * HG, HG), HG), :] = o8 / l_s[z]

        start_k(0, 1)

        def heads(w_v, s, q):
            return jnp.swapaxes(w_v[s].reshape(128, H, D)[:, q * HQ:(q + 1) * HQ, :], 0, 1)

        def side_v(g, u, q):
            lanes = slice(q * HQ * D, (q + 1) * HQ * D)

            @pl.when(g == 1)
            def _():
                wt = heads(wqa_v, u, q)
                w = jnp.concatenate([wt[h] for h in range(HQ)], axis=-1)
                qa_s[:, lanes] += _dot(xs[u].astype(BF16), w)

            @pl.when(g == 2)
            def _():
                wt = heads(wuk_v, u, q)
                qa = qa_s[:, lanes].astype(BF16)
                t = jnp.stack([_dot_nt(qa[:, h * D:(h + 1) * D], wt[h]) for h in range(HQ)])
                qabs_s[u, :, q * HQ:(q + 1) * HQ, :] = jnp.swapaxes(t, 0, 1)

            r0 = ((((g - 3) & 3) * 4 + u) * NQ + q) * 128

            @pl.when(jnp.logical_and(g >= 3, g < 7))
            def _():
                qk(r0, 1)

            @pl.when(jnp.logical_and(g >= 7, g < 11))
            def _():
                if q == 0:
                    pl.when(r0 == 0)(lambda: softmax(1))
                pv(r0, 1)

            @pl.when(g == 12)
            def _():
                wt = heads(wuv_v, u, q)
                c = jnp.swapaxes(ctxc_s[u, :, q * HQ:(q + 1) * HQ, :], 0, 1).astype(BF16)
                ctx_s[:, lanes] += jnp.concatenate([_dot(c[h], wt[h]) for h in range(HQ)], axis=-1)

            @pl.when(g == NG - 1)
            def _():
                outb_s[...] += _dot(ol_s[u, :, q * CQ:(q + 1) * CQ].astype(BF16), wob_v[u, q * CQ:(q + 1) * CQ, :])

        def side_k(g, u, q):
            ab = jnp.clip((g - 3) >> 1, 0, B - 1)
            act = jnp.logical_and(g >= 3, g < 11)
            keys = slice(q * CQ, (q + 1) * CQ)

            @pl.when(jnp.logical_and(act, (g & 1) == 1))
            def _():
                qc = jnp.concatenate([qabs_s[s, ab] for s in range(4)], axis=-1).astype(BF16)
                s = _dot_nt(qc, ckv_v[ab * 4 + u, keys, :])
                sa_s[u, :, keys] = s
                m = s[:, 0:128]
                for i in range(1, CQ // 128):
                    m = jnp.maximum(m, s[:, i * 128:(i + 1) * 128])
                mo = jnp.maximum(m, ma_s[...])
                ma_s[...] = jnp.where(u == 0, m, mo) if q == 0 else mo

            @pl.when(jnp.logical_and(act, (g & 1) == 0))
            def _():
                if q == 0:
                    @pl.when(u == 0)
                    def _():
                        ma_s[...] = jnp.broadcast_to(jnp.max(ma_s[...], axis=-1, keepdims=True), ma_s.shape)
                        la_s[...] = jnp.zeros(la_s.shape, F32)
                        acca_s[...] = jnp.zeros(acca_s.shape, F32)
                m = ma_s[...]
                p = jnp.exp((sa_s[u, :, keys] - jnp.concatenate([m] * (CQ // 128), axis=-1)) * SCALE)
                l = la_s[...]
                for i in range(CQ // 128):
                    l = l + p[:, i * 128:(i + 1) * 128]
                la_s[...] = l
                acca_s[...] += _dot(p.astype(BF16), ckv_v[ab * 4 + u, keys, :])
                if q == NQ - 1:
                    @pl.when(u == 3)
                    def _():
                        c = acca_s[...] / jnp.sum(la_s[...], axis=-1, keepdims=True)
                        for s in range(4):
                            ctxc_s[s, ab] = c[:, s * 128:(s + 1) * 128]

            if q == 0:
                pl.when(jnp.logical_and(g == 11, u == 0))(lambda: finish_v(0, 1))

                @pl.when(jnp.logical_and(g == NG - 1, u == 0))
                def _():
                    of_s[NU - ROLL:NU, :] = o_s[0:ROLL, :]
                    of_s[0:NU - ROLL, :] = o_s[ROLL:NU, :]
                    t = jnp.swapaxes(of_s[...].reshape(8, H, D), 0, 1)
                    for hg in range(4):
                        ol_s[hg] = jnp.concatenate([t[hg * 8 + h] for h in range(8)], axis=-1)

        def phase(a, g):
            cur = kv(a, g)
            if a == 0:
                nxts = [(None, kv(1, g))]
                start_k(g)
            else:
                nxts = [(g < NG - 1, kv(0, jnp.minimum(g + 1, NG - 1))), (g == NG - 1, last)]
            work = pv if a else qk
            sched = dict(SCHED)

            def group(u, c):
                for t in range(GP):
                    point(cur, u * 8 + t // NP, t % NP, nxts, DT, h_in_cur=t + HS < GP, h_next=t + HS - GP)
                    item = sched.get(t + 1)
                    if item is None:
                        continue
                    i = int(item[1])
                    if item[0] == "A":
                        (side_v if a else side_k)(g, u, i)
                    elif item[0] == "L":
                        assert (i + 1) * 128 <= (t + 1) // NP * 80 + sum(_Rows.pat[:(t + 1) % NP])
                        work(cur.parts[0].lo_tile(u, i))
                    else:
                        assert t + 1 >= 8 * i
                        cur.hi_wait((u * 3 + i) * 8, 8)
                        work(cur.parts[0].hi_tile(u, i))
                return c
            lax.fori_loop(0, 4, group, 0)
            if a == 0:
                softmax()
            else:
                finish_v(g)

        def body(g, c):
            phase(0, g)
            phase(1, g)
            return c
        lax.fori_loop(1, NG, body, 0)

        def lhs(rows, n):
            return jnp.concatenate([ctx_s[:, s * 1024 + r:s * 1024 + r + n] for r in rows for s in range(4)],
                                   axis=-1).astype(BF16)

        def rhs(rows, n):
            return jnp.concatenate([woa_v[s, r:r + n, :] for r in rows for s in range(4)], axis=0)

        full = {11: 0, 15: 640, 20: 128, 29: 256, 33: 768, 38: 384}
        qrow = {n: 512 + 32 * i for i, n in enumerate("abcd")}
        qrow.update({n: 896 + 32 * i for i, n in enumerate("efgh")})
        tail = dict(TAIL)
        tail_lhs = {}
        acc = None
        for t in range(1, 16 * NP + 1):
            point(last, (t - 1) // NP, (t - 1) % NP, [], DT)
            arrived = t // NP * 40 + sum(_Last.pat[:t % NP])
            if t == 3:
                u0 = NU - HG - ROLL
                assert u0 // H == (u0 + HG - 1) // H
                o = jnp.where(blk, acc_s[0] / l_s[0][:, 0:1], 0.0)
                o = jnp.sum(o, axis=0, keepdims=True)
                rowb = lax.broadcasted_iota(jnp.int32, (8, HG * D), 0) == u0 // H
                o = jnp.where(rowb, jnp.broadcast_to(o, (8, HG * D)), 0.0)
                h0 = u0 % H
                w = jnp.concatenate([wob_v[h // 8, (h % 8) * D:(h % 8 + 1) * D, :] for h in range(h0, h0 + HG)], axis=0)
                out_ref[:, M:] = (outb_s[...] + _dot(o.astype(BF16), w))[0:B, :].astype(out_ref.dtype)
            if t == 24:
                tail_lhs = {tt: lhs([qrow[n] for n in names], 32) for tt, names in TAIL}
            if t in full:
                r = full[t]
                if r >= 640:
                    last.hi_wait((r - 640) // 8, 16)
                else:
                    assert r + 128 <= arrived
                d = _dot(lhs([r], 128), rhs([r], 128))
                acc = d if acc is None else acc + d
            if t in tail:
                for n in tail[t]:
                    if qrow[n] >= 640:
                        last.hi_wait((qrow[n] - 640) // 8, 4)
                    else:
                        assert qrow[n] + 32 <= arrived
                acc = acc + _dot(tail_lhs[t], rhs([qrow[n] for n in tail[t]], 32))
        out_ref[:, :M] = acc[0:B, :].astype(out_ref.dtype)

    scratch = [
        pltpu.VMEM((2, HG, SK, D), BF16), pltpu.VMEM((2, HG, SK, D), BF16),
        pltpu.VMEM((4, 128, H * D), BF16),
        pltpu.VMEM((4, 4096, D), BF16), pltpu.VMEM((4, 4096, D), BF16), pltpu.VMEM((4, 4096, D), BF16),
        pltpu.VMEM((16, 1024, DC), BF16),
        pltpu.VMEM((4, 1024, M), BF16), pltpu.VMEM((4, 1024, M), BF16),
        pltpu.VMEM((B, M), BF16), pltpu.VMEM((B, M), BF16),
        pltpu.VMEM((8, 8, 128), F32),
        pltpu.VMEM((NU, D), F32),
        pltpu.VMEM((NU, D), F32),
        pltpu.VMEM((2, 8, HG * D), F32),
        pltpu.VMEM((2, 32, 8, 128), F32),
        pltpu.VMEM((2, 8, 128), F32),
        pltpu.VMEM((2, 8, HG * D), F32),
        pltpu.VMEM((NU, D), F32),
        pltpu.VMEM((8 * H, D), F32),
        pltpu.VMEM((4, 8, HG * D), F32),
        pltpu.VMEM((8, H * D), F32),
        pltpu.VMEM((4, 8, H, 128), F32),
        pltpu.VMEM((4, H, 1024), F32),
        pltpu.VMEM((H, 128), F32),
        pltpu.VMEM((H, 128), F32),
        pltpu.VMEM((H, DC), F32),
        pltpu.VMEM((4, 8, H, 128), F32),
        pltpu.VMEM((8, H * D), F32),
        pltpu.VMEM((8, M), F32),
        pltpu.SemaphoreType.DMA((16 * NP,)),
        pltpu.SemaphoreType.DMA((8,)),
        pltpu.SemaphoreType.DMA((6,)),
        pltpu.SemaphoreType.DMA((2,)),
        pltpu.SemaphoreType.DMA((6,)),
    ]

    @jax.jit
    def fn(A_x, A_c_kv, A_w_q, A_w_uk, A_w_uv, A_w_o, B_x, B_k_cache, B_v_cache, B_wq, B_wo):
        out = pl.pallas_call(
            kernel,
            in_specs=[pl.BlockSpec(memory_space=pl.ANY)] * 11,
            out_specs=pl.BlockSpec(memory_space=pltpu.VMEM),
            out_shape=jax.ShapeDtypeStruct((B, 2 * M), BF16),
            scratch_shapes=scratch,
            compiler_params=pltpu.CompilerParams(vmem_limit_bytes=100 * 1024 * 1024, disable_bounds_checks=not checks,
                                                 disable_semaphore_checks=not checks),
            name="fused_decode",
        )(A_x.reshape(B, M), A_c_kv.reshape(16, 1024, DC), A_w_q.reshape(4, 4096, D), A_w_uk.reshape(4, 4096, D),
          A_w_uv.reshape(4, 4096, D), A_w_o.reshape(4, 1024, M), B_x.reshape(B, M),
          B_k_cache.reshape(NU, SK, D), B_v_cache.reshape(NU, SK, D),
          B_wq.reshape(4, 128, H * D), B_wo.reshape(4, 1024, M))
        return out.reshape(B, 1, 2 * M)

    return fn


_fn = make_kernel()


@jax.jit
def pallas_concat_heads__compressed_kv_cla__mha_block_cached__decode_kernel(
    A_x: jax.Array,
    A_c_kv: jax.Array,
    A_w_q: jax.Array,
    A_w_uk: jax.Array,
    A_w_uv: jax.Array,
    A_w_o: jax.Array,
    B_x: jax.Array,
    B_k_cache: jax.Array,
    B_v_cache: jax.Array,
    B_wq: jax.Array,
    B_wo: jax.Array,
):
    return _fn(A_x, A_c_kv, A_w_q, A_w_uk, A_w_uv, A_w_o, B_x, B_k_cache, B_v_cache, B_wq, B_wo)
```

```python
import jax
import jax.numpy as jnp
from jax import lax
import jax.experimental.pallas as pl
import jax.experimental.pallas.tpu as pltpu

B, H, SK, D, M = 4, 32, 4096, 128, 512
DC = 512
HG = 8
NU = B * H
NG = NU // HG
F32 = jnp.float32
BF16 = jnp.bfloat16
LO, HI = 1, 0
SCALE = D ** -0.5
NP = 3
HS = 8
PHI = 2
ROLL = HG - PHI
ALL = slice(None)


def _dot(a, b):
    return jnp.dot(a, b, preferred_element_type=F32)


def _dot_nt(a, b):
    return lax.dot_general(a, b, (((1,), (1,)), ((), ())), preferred_element_type=F32)


def _mo(x, n):
    return x if isinstance(x, int) else pl.multiple_of(x, n)


def _sel(c, a, b):
    return (a if c else b) if isinstance(c, bool) else jnp.where(c, a, b)


class _Rows:
    ntr = 32
    pat = (24, 24, 32)
    UP_UP = ((0, 1), (2816, 1), (2048, 1), (1280, 1))
    UP_DOWN = ((0, 1), (3328, -1), (4096, -1), (1280, 1))

    def __init__(self, src, dst, walk):
        self.src, self.dst, self.walk = src, dst, walk

    def _row(self, first, seg, off, half, n):
        def pos(s, o):
            return s[0] + o if s[1] > 0 else s[0] - o - n
        return _sel(first, pos(self.walk[seg], off), pos(self.walk[seg + 1], off - half))

    def lo(self, tr, k, odd=None):
        r = self._row(tr < 16, 0, tr * 80 + sum(self.pat[:k]), 1280, self.pat[k])
        return ALL, pl.ds(_mo(r, 8), self.pat[k])

    def hi(self, j, n=1):
        return ALL, pl.ds(_mo(self._row(j < 48, 2, j * 16, 768, n * 16), 8), n * 16)

    def hi_all(self):
        assert self.walk == self.UP_UP
        return ALL, pl.ds(1280, 1536)

    def lo_tile(self, u, i):
        return self._row(u < 2, 0, (u * 5 + i) * 128, 1280, 128)

    def hi_tile(self, u, i):
        return self._row(u < 2, 2, (u * 3 + i) * 128, 768, 128)


class _Cells:
    ntr = 32

    def __init__(self, src, dst, lg):
        self.src, self.dst, self.lg = src, dst, lg

    def _idx(self, c, off, width):
        return (ALL, pl.ds(_mo((c >> self.lg) * 8, 8), 8),
                pl.ds(_mo((c & ((1 << self.lg) - 1)) * 512 + off, 128), width))

    def lo(self, tr, k, odd):
        c = (tr >> 1) * 5 + (tr >> 4) * 48 + 2 * odd + k
        if k == 2 - 2 * odd:
            return self._idx(c, odd * 256, 256)
        return self._idx(c, 0, 512)

    def hi(self, j):
        hc = j + _sel(j < 48, 128, 32)
        return self._idx(hc >> 1, (hc & 1) * 256, 256)

    def hi_all(self):
        return ALL, pl.ds((40 >> self.lg) * 8, (48 >> self.lg) * 8)


class _Last:
    ntr = 16
    pat = (16, 16, 8)

    def __init__(self, src, dst):
        self.src, self.dst = src, dst

    def lo(self, tr, k, odd=None):
        return ALL, pl.ds(_mo(tr * 40 + sum(self.pat[:k]), 8), self.pat[k])

    def hi(self, j, n=1):
        return ALL, pl.ds(640 + j * 8, n * 8)


class _Block:
    def __init__(self, parts, hsem):
        self.parts, self.hsem, self.ntr = parts, hsem, parts[0].ntr

    def _copies(self, idx, sem):
        return [pltpu.make_async_copy(p.src.at[idx(p)], p.dst.at[idx(p)], sem(i)) for i, p in enumerate(self.parts)]

    def lo_start(self, tr, k, sem, odd=None):
        for c in self._copies(lambda p: p.lo(tr, k, odd), lambda i: sem):
            c.start(priority=LO)

    def lo_wait(self, tr, k, sem, odd=None):
        for c in self._copies(lambda p: p.lo(tr, k, odd), lambda i: sem):
            c.wait()

    def hi_start(self, j):
        for c in self._copies(lambda p: p.hi(j), lambda i: self.hsem(j, i)):
            c.start(priority=HI)

    def hi_wait(self, j, n):
        for c in self._copies(lambda p: p.hi(j, n), lambda i: self.hsem(j, i)):
            c.wait()

    def hi_wait_all(self):
        for c in self._copies(lambda p: p.hi_all(), lambda i: self.hsem(0, i)):
            c.wait()


def make_kernel(DT=12, DTP=5, checks=False,
                SCHED=((2, "A0"), (5, "L0"), (8, "H0"), (10, "L1"), (13, "A1"), (15, "L2"), (17, "H1"), (20, "L3"),
                       (22, "H2"), (24, "L4")),
                TAIL=((39, "ef"), (44, "abg"), (48, "cdh"))):
    assert DTP <= DT < 16
    NQ = 2
    HQ = H // (2 * NQ)
    CQ = 1024 // NQ
    GP = 8 * NP

    def kernel(xa_h, ckv_h, wqa_h, wuk_h, wuv_h, woa_h, xb_h, k_h, v_h, wqb_h, wob_h,
               out_ref,
               kbuf, vbuf, wqb_v, wqa_v, wuk_v, wuv_v, ckv_v, woa_v, wob_v, xa_v, xb_v,
               xs, qf_s, q_s, qm_s, s_s, m_s, l_s, acc_s, o_s, of_s, ol_s,
               qa_s, qabs_s, sa_s, ma_s, la_s, acca_s, ctxc_s, ctx_s, outb_s,
               lsem, hsem, esem, xsem, tsem):

        def kv(a, g):
            src, dst = (k_h, v_h)[a], (kbuf, vbuf)[a]
            return _Block([_Rows(src.at[pl.ds(g * HG - ROLL, HG)], dst.at[0], _Rows.UP_DOWN)],
                          lambda j, i: hsem.at[a * 4 + ((j >> 3) & 3)])

        def part(src, dst, u0, n, d0=None):
            s, d = src.at[pl.ds(u0, n)], dst.at[pl.ds(u0 if d0 is None else d0, n)]
            lanes = src.shape[-1]
            return _Rows(s, d, _Rows.UP_UP) if lanes == 128 else _Cells(s, d, 0 if lanes == 512 else 3)

        k0, v0 = kbuf.at[1], vbuf.at[1]
        pre = [
            [part(wob_h, wob_v, 2, 2), part(wqb_h, wqb_v, 0, 4), part(v_h, v0, 0, PHI, ROLL)],
            [part(wuk_h, wuk_v, 2, 2), part(wqa_h, wqa_v, 0, 4), part(ckv_h, ckv_v, 0, 2)],
            [part(wuv_h, wuv_v, 0, 4), part(wuk_h, wuk_v, 0, 2)],
            [part(ckv_h, ckv_v, 2, 8)],
            [part(ckv_h, ckv_v, 10, 6)],
            [part(k_h, k0, NU - ROLL, ROLL, 0), part(wob_h, wob_v, 0, 2)],
            [part(v_h, v0, NU - ROLL, ROLL, 0), part(k_h, k0, 0, PHI, ROLL)],
        ]
        pre = [_Block(p, lambda j, i, n=n: esem.at[(n & 1) * 3 + i]) for n, p in enumerate(pre)]
        last = _Block([_Last(woa_h, woa_v)], lambda j, i: tsem.at[j // 16 if j < 32 else 2 + (j - 32) // 4])

        def lsem_at(tr, k):
            return lsem.at[(tr & 15) * NP + k]

        def either(pos, lim, cur_fn, nxts, nxt_fn):
            if isinstance(pos, int):
                if pos < lim:
                    cur_fn()
                else:
                    assert not nxts
                return
            pl.when(pos < lim)(cur_fn)
            for cond, nxt in nxts:
                c = pos >= lim
                if cond is not None:
                    c = jnp.logical_and(c, cond)
                pl.when(c)(lambda nxt=nxt: nxt_fn(nxt))

        def point(cur, tr, k, nxts, dt, odd=0, h_in_cur=False, h_next=None):
            j = tr * NP + k + HS
            nj = NP * cur.ntr
            if h_in_cur:
                cur.hi_start(j)
            else:
                either(j, nj, lambda: cur.hi_start(j), nxts,
                       lambda nxt: nxt.hi_start(j - nj if h_next is None else h_next))
            cur.lo_wait(tr, k, lsem_at(tr, k), odd)
            ta, oa = tr + dt, (odd + dt) & 1
            sem = lsem_at(ta, k)
            either(ta, cur.ntr, lambda: cur.lo_start(ta, k, sem, oa), nxts,
                   lambda nxt: nxt.lo_start(ta - cur.ntr, k, sem, oa))

        def stream(cur, nxt, extra=None):
            def body(m, c):
                for odd in range(2):
                    for k in range(NP):
                        point(cur, m * 2 + odd, k, [(None, nxt)], DTP, odd)
                if extra is not None:
                    extra(m)
                return c
            lax.fori_loop(0, cur.ntr // 2, body, 0)
            cur.hi_wait_all()

        zeroed = [[xs, o_s, qa_s], [of_s, ctx_s, outb_s, ma_s], [ctxc_s.at[0], ctxc_s.at[1]], [ctxc_s.at[2], ctxc_s.at[3]]]
        xb_cp = pltpu.make_async_copy(xb_h, xb_v, xsem.at[0])
        xa_cp = pltpu.make_async_copy(xa_h, xa_v, xsem.at[1])
        for j in range(HS):
            if j < DTP:
                for k in range(NP):
                    pre[0].lo_start(j, k, lsem_at(j, k), j & 1)
            pre[0].hi_start(j)
            if j == 2:
                xb_cp.start(priority=HI)
                xa_cp.start(priority=HI)
            if j >= HS - len(zeroed):
                for r in zeroed[j - HS]:
                    r[...] = jnp.zeros(r.shape, F32)
        assert DTP <= HS

        stream(pre[0], pre[1])

        xb_cp.wait()
        xa_cp.wait()
        for s in range(4):
            xs[s, 0:B, :] = xa_v[:, s * 128:(s + 1) * 128].astype(F32)
            xs[4 + s, 0:B, :] = xb_v[:, s * 128:(s + 1) * 128].astype(F32)

        def qb_piece(m):
            @pl.when((m & 3) == 1)
            def _():
                hg = m >> 2
                x = jnp.concatenate([xs[4 + s] for s in range(4)], axis=-1).astype(BF16)
                w = wqb_v[:, :, pl.ds(pl.multiple_of(hg * 1024, 1024), 1024)].reshape(M, 1024)
                q = _dot(x, w)
                q = jnp.swapaxes(jnp.stack([q[:, h * D:(h + 1) * D] for h in range(8)]), 0, 1)
                for b in range(B):
                    qf_s[pl.ds(pl.multiple_of(b * H + hg * 8, 8), 8), :] = q[b]

        stream(pre[1], pre[2], qb_piece)
        q_s[0:ROLL, :] = qf_s[NU - ROLL:NU, :]
        q_s[ROLL:NU, :] = qf_s[0:NU - ROLL, :]
        for n in range(2, len(pre)):
            stream(pre[n], pre[n + 1] if n + 1 < len(pre) else kv(0, 1))

        def deepen(tr, c):
            for k in range(NP):
                kv(0, 1).lo_start(tr, k, lsem_at(tr, k))
            return c
        lax.fori_loop(DTP, DT, deepen, 0)

        blk = (lax.broadcasted_iota(jnp.int32, (8, HG * D), 1) >> 7) == lax.broadcasted_iota(jnp.int32, (8, HG * D), 0)

        def tile(buf, z, r):
            r = pl.multiple_of(r, 128)
            return jnp.concatenate([buf[z, i, pl.ds(r, 128), :] for i in range(HG)], axis=-1)

        def start_k(g, z=0):
            q = q_s[pl.ds(_mo(g * HG, HG), HG), :]
            qm_s[z] = jnp.where(blk, jnp.concatenate([q] * HG, axis=-1), 0.0)
            m_s[z] = jnp.full((8, 128), -jnp.inf, F32)

        def qk(r, z=0):
            s = _dot_nt(qm_s[z].astype(BF16), tile(kbuf, z, r))
            s_s[z, r >> 7] = s
            m_s[z] = jnp.maximum(m_s[z], s)

        def start_v(z=0):
            m_s[z] = jnp.broadcast_to(jnp.max(m_s[z], axis=-1, keepdims=True), (8, 128))
            l_s[z] = jnp.zeros((8, 128), F32)
            acc_s[z] = jnp.zeros((8, HG * D), F32)

        def pv(r, z=0):
            p = jnp.exp((s_s[z, r >> 7] - m_s[z]) * SCALE)
            l_s[z] += p
            acc_s[z] += _dot(p.astype(BF16), tile(vbuf, z, r))

        def finish_v(g, z=0):
            o = jnp.where(blk, acc_s[z], 0.0)
            o8 = o[:, 0:D]
            for i in range(1, HG):
                o8 = o8 + o[:, i * D:(i + 1) * D]
            o_s[pl.ds(_mo(g * HG, HG), HG), :] = o8 / jnp.sum(l_s[z], axis=-1, keepdims=True)

        start_k(0, 1)

        def heads(w_v, s, q):
            return jnp.swapaxes(w_v[s].reshape(128, H, D)[:, q * HQ:(q + 1) * HQ, :], 0, 1)

        def side_proj(g, u, q):
            lanes = slice(q * HQ * D, (q + 1) * HQ * D)

            @pl.when(g == 1)
            def _():
                wt = heads(wqa_v, u, q)
                w = jnp.concatenate([wt[h] for h in range(HQ)], axis=-1)
                qa_s[:, lanes] += _dot(xs[u].astype(BF16), w)

            @pl.when(g == 2)
            def _():
                wt = heads(wuk_v, u, q)
                qa = qa_s[:, lanes].astype(BF16)
                t = jnp.stack([_dot_nt(qa[:, h * D:(h + 1) * D], wt[h]) for h in range(HQ)])
                qabs_s[u, :, q * HQ:(q + 1) * HQ, :] = jnp.swapaxes(t, 0, 1)

            @pl.when(g == 12)
            def _():
                wt = heads(wuv_v, u, q)
                c = jnp.swapaxes(ctxc_s[u, :, q * HQ:(q + 1) * HQ, :], 0, 1).astype(BF16)
                ctx_s[:, lanes] += jnp.concatenate([_dot(c[h], wt[h]) for h in range(HQ)], axis=-1)

        def side_v(g, u, q):
            side_proj(g, u, NQ + q)
            r0 = ((((g - 3) & 3) * 4 + u) * NQ + q) * 128

            @pl.when(jnp.logical_and(g >= 3, g < 7))
            def _():
                qk(r0, 1)

            @pl.when(jnp.logical_and(g >= 7, g < 11))
            def _():
                if q == 0:
                    pl.when(r0 == 0)(lambda: start_v(1))
                pv(r0, 1)

            @pl.when(g == NG - 1)
            def _():
                outb_s[...] += _dot(ol_s[u, :, q * CQ:(q + 1) * CQ].astype(BF16), wob_v[u, q * CQ:(q + 1) * CQ, :])

        def side_k(g, u, q):
            side_proj(g, u, q)
            ab = jnp.clip((g - 3) >> 1, 0, B - 1)
            act = jnp.logical_and(g >= 3, g < 11)
            keys = slice(q * CQ, (q + 1) * CQ)

            @pl.when(jnp.logical_and(act, (g & 1) == 1))
            def _():
                qc = jnp.concatenate([qabs_s[s, ab] for s in range(4)], axis=-1).astype(BF16)
                s = _dot_nt(qc, ckv_v[ab * 4 + u, keys, :])
                sa_s[u, :, keys] = s
                m = s[:, 0:128]
                for i in range(1, CQ // 128):
                    m = jnp.maximum(m, s[:, i * 128:(i + 1) * 128])
                mo = jnp.maximum(m, ma_s[...])
                ma_s[...] = jnp.where(u == 0, m, mo) if q == 0 else mo

            @pl.when(jnp.logical_and(act, (g & 1) == 0))
            def _():
                if q == 0:
                    @pl.when(u == 0)
                    def _():
                        ma_s[...] = jnp.broadcast_to(jnp.max(ma_s[...], axis=-1, keepdims=True), ma_s.shape)
                        la_s[...] = jnp.zeros(la_s.shape, F32)
                        acca_s[...] = jnp.zeros(acca_s.shape, F32)
                m = ma_s[...]
                p = jnp.exp((sa_s[u, :, keys] - jnp.concatenate([m] * (CQ // 128), axis=-1)) * SCALE)
                l = la_s[...]
                for i in range(CQ // 128):
                    l = l + p[:, i * 128:(i + 1) * 128]
                la_s[...] = l
                acca_s[...] += _dot(p.astype(BF16), ckv_v[ab * 4 + u, keys, :])
                if q == NQ - 1:
                    @pl.when(u == 3)
                    def _():
                        c = acca_s[...] / jnp.sum(la_s[...], axis=-1, keepdims=True)
                        for s in range(4):
                            ctxc_s[s, ab] = c[:, s * 128:(s + 1) * 128]

            if q == 0:
                pl.when(jnp.logical_and(g == 11, u == 0))(lambda: finish_v(0, 1))

                @pl.when(jnp.logical_and(g == NG - 1, u == 0))
                def _():
                    of_s[NU - ROLL:NU, :] = o_s[0:ROLL, :]
                    of_s[0:NU - ROLL, :] = o_s[ROLL:NU, :]
                    t = jnp.swapaxes(of_s[...].reshape(8, H, D), 0, 1)
                    for hg in range(4):
                        ol_s[hg] = jnp.concatenate([t[hg * 8 + h] for h in range(8)], axis=-1)

        def phase(a, g):
            cur = kv(a, g)
            if a == 0:
                nxts = [(None, kv(1, g))]
                start_k(g)
            else:
                nxts = [(g < NG - 1, kv(0, jnp.minimum(g + 1, NG - 1))), (g == NG - 1, last)]
            work = pv if a else qk
            sched = dict(SCHED)

            def group(u, c):
                for t in range(GP):
                    point(cur, u * 8 + t // NP, t % NP, nxts, DT, h_in_cur=t + HS < GP, h_next=t + HS - GP)
                    item = sched.get(t + 1)
                    if item is None:
                        continue
                    i = int(item[1])
                    if item[0] == "A":
                        (side_v if a else side_k)(g, u, i)
                    elif item[0] == "L":
                        assert (i + 1) * 128 <= (t + 1) // NP * 80 + sum(_Rows.pat[:(t + 1) % NP])
                        work(cur.parts[0].lo_tile(u, i))
                    else:
                        assert t + 1 >= 8 * i
                        cur.hi_wait((u * 3 + i) * 8, 8)
                        work(cur.parts[0].hi_tile(u, i))
                return c
            lax.fori_loop(0, 4, group, 0)
            if a == 0:
                start_v()
            else:
                finish_v(g)

        def body(g, c):
            phase(0, g)
            phase(1, g)
            return c
        lax.fori_loop(1, NG, body, 0)

        def lhs(rows, n):
            return jnp.concatenate([ctx_s[:, s * 1024 + r:s * 1024 + r + n] for r in rows for s in range(4)],
                                   axis=-1).astype(BF16)

        def rhs(rows, n):
            return jnp.concatenate([woa_v[s, r:r + n, :] for r in rows for s in range(4)], axis=0)

        full = {11: 0, 15: 640, 20: 128, 29: 256, 33: 768, 38: 384}
        qrow = {n: 512 + 32 * i for i, n in enumerate("abcd")}
        qrow.update({n: 896 + 32 * i for i, n in enumerate("efgh")})
        tail = dict(TAIL)
        tail_lhs = {}
        acc = None
        for t in range(1, 16 * NP + 1):
            point(last, (t - 1) // NP, (t - 1) % NP, [], DT)
            arrived = t // NP * 40 + sum(_Last.pat[:t % NP])
            if t == 3:
                u0 = NU - HG - ROLL
                assert u0 // H == (u0 + HG - 1) // H
                o = jnp.where(blk, acc_s[0] / jnp.sum(l_s[0], axis=-1, keepdims=True), 0.0)
                o = jnp.sum(o, axis=0, keepdims=True)
                rowb = lax.broadcasted_iota(jnp.int32, (8, HG * D), 0) == u0 // H
                o = jnp.where(rowb, jnp.broadcast_to(o, (8, HG * D)), 0.0)
                h0 = u0 % H
                w = jnp.concatenate([wob_v[h // 8, (h % 8) * D:(h % 8 + 1) * D, :] for h in range(h0, h0 + HG)], axis=0)
                out_ref[:, M:] = (outb_s[...] + _dot(o.astype(BF16), w))[0:B, :].astype(out_ref.dtype)
            if t == 24:
                tail_lhs = {tt: lhs([qrow[n] for n in names], 32) for tt, names in TAIL}
            if t in full:
                r = full[t]
                if r >= 640:
                    last.hi_wait((r - 640) // 8, 16)
                else:
                    assert r + 128 <= arrived
                d = _dot(lhs([r], 128), rhs([r], 128))
                acc = d if acc is None else acc + d
            if t in tail:
                for n in tail[t]:
                    if qrow[n] >= 640:
                        last.hi_wait((qrow[n] - 640) // 8, 4)
                    else:
                        assert qrow[n] + 32 <= arrived
                acc = acc + _dot(tail_lhs[t], rhs([qrow[n] for n in tail[t]], 32))
        out_ref[:, :M] = acc[0:B, :].astype(out_ref.dtype)

    scratch = [
        pltpu.VMEM((2, HG, SK, D), BF16), pltpu.VMEM((2, HG, SK, D), BF16),
        pltpu.VMEM((4, 128, H * D), BF16),
        pltpu.VMEM((4, 4096, D), BF16), pltpu.VMEM((4, 4096, D), BF16), pltpu.VMEM((4, 4096, D), BF16),
        pltpu.VMEM((16, 1024, DC), BF16),
        pltpu.VMEM((4, 1024, M), BF16), pltpu.VMEM((4, 1024, M), BF16),
        pltpu.VMEM((B, M), BF16), pltpu.VMEM((B, M), BF16),
        pltpu.VMEM((8, 8, 128), F32),
        pltpu.VMEM((NU, D), F32),
        pltpu.VMEM((NU, D), F32),
        pltpu.VMEM((2, 8, HG * D), F32),
        pltpu.VMEM((2, 32, 8, 128), F32),
        pltpu.VMEM((2, 8, 128), F32),
        pltpu.VMEM((2, 8, 128), F32),
        pltpu.VMEM((2, 8, HG * D), F32),
        pltpu.VMEM((NU, D), F32),
        pltpu.VMEM((8 * H, D), F32),
        pltpu.VMEM((4, 8, HG * D), F32),
        pltpu.VMEM((8, H * D), F32),
        pltpu.VMEM((4, 8, H, 128), F32),
        pltpu.VMEM((4, H, 1024), F32),
        pltpu.VMEM((H, 128), F32),
        pltpu.VMEM((H, 128), F32),
        pltpu.VMEM((H, DC), F32),
        pltpu.VMEM((4, 8, H, 128), F32),
        pltpu.VMEM((8, H * D), F32),
        pltpu.VMEM((8, M), F32),
        pltpu.SemaphoreType.DMA((16 * NP,)),
        pltpu.SemaphoreType.DMA((8,)),
        pltpu.SemaphoreType.DMA((6,)),
        pltpu.SemaphoreType.DMA((2,)),
        pltpu.SemaphoreType.DMA((6,)),
    ]

    @jax.jit
    def fn(A_x, A_c_kv, A_w_q, A_w_uk, A_w_uv, A_w_o, B_x, B_k_cache, B_v_cache, B_wq, B_wo):
        out = pl.pallas_call(
            kernel,
            in_specs=[pl.BlockSpec(memory_space=pl.ANY)] * 11,
            out_specs=pl.BlockSpec(memory_space=pltpu.VMEM),
            out_shape=jax.ShapeDtypeStruct((B, 2 * M), BF16),
            scratch_shapes=scratch,
            compiler_params=pltpu.CompilerParams(vmem_limit_bytes=100 * 1024 * 1024, disable_bounds_checks=not checks,
                                                 disable_semaphore_checks=not checks),
            name="fused_decode",
        )(A_x.reshape(B, M), A_c_kv.reshape(16, 1024, DC), A_w_q.reshape(4, 4096, D), A_w_uk.reshape(4, 4096, D),
          A_w_uv.reshape(4, 4096, D), A_w_o.reshape(4, 1024, M), B_x.reshape(B, M),
          B_k_cache.reshape(NU, SK, D), B_v_cache.reshape(NU, SK, D),
          B_wq.reshape(4, 128, H * D), B_wo.reshape(4, 1024, M))
        return out.reshape(B, 1, 2 * M)

    return fn


_fn = make_kernel()


@jax.jit
def pallas_concat_heads__compressed_kv_cla__mha_block_cached__decode_kernel(
    A_x: jax.Array,
    A_c_kv: jax.Array,
    A_w_q: jax.Array,
    A_w_uk: jax.Array,
    A_w_uv: jax.Array,
    A_w_o: jax.Array,
    B_x: jax.Array,
    B_k_cache: jax.Array,
    B_v_cache: jax.Array,
    B_wq: jax.Array,
    B_wo: jax.Array,
):
    return _fn(A_x, A_c_kv, A_w_q, A_w_uk, A_w_uv, A_w_o, B_x, B_k_cache, B_v_cache, B_wq, B_wo)
```

```python
import jax
import jax.numpy as jnp
from jax import lax
import jax.experimental.pallas as pl
import jax.experimental.pallas.tpu as pltpu

B, H, SK, D, M = 4, 32, 4096, 128, 512
DC = 512
NU = B * H
NG = NU // 16
PHI = 2
F32 = jnp.float32
BF16 = jnp.bfloat16
LO, HI = 1, 0
SCALE = D ** -0.5
ALL = slice(None)


def _dot(a, b):
    return jnp.dot(a, b, preferred_element_type=F32)


def _dot_nt(a, b):
    return lax.dot_general(a, b, (((1,), (1,)), ((), ())), preferred_element_type=F32)


def _mo(x, n):
    return x if isinstance(x, int) else pl.multiple_of(x, n)


class _Part:
    def __init__(self, src, dst, s0, n, d0=None, width=128):
        self.src = src.at[pl.ds(s0, n)]
        self.dst = dst.at[pl.ds(s0 if d0 is None else d0, n)]
        self.lg = (src.shape[-1] // width).bit_length() - 1
        self.width = width

    def copy(self, j, n, sem):
        if j is None:
            idx = (ALL,)
        elif self.lg == 0:
            idx = (ALL, pl.ds(_mo(j * 8, 8), n * 8))
        else:
            assert n == 1
            idx = (ALL, pl.ds(_mo((j >> self.lg) * 8, 8), 8),
                   pl.ds(_mo((j & ((1 << self.lg) - 1)) * self.width, 128), self.width))
        return pltpu.make_async_copy(self.src.at[idx], self.dst.at[idx], sem)


class _Block:
    def __init__(self, lo, hi, hsem, npts=256):
        self.lo, self.hi, self.hsem, self.npts = lo, hi, hsem, npts

    def lo_start(self, j, sem):
        for p in self.lo:
            p.copy(j, 1, sem).start(priority=LO)

    def lo_wait(self, j, sem):
        for p in self.lo:
            p.copy(j, 1, sem).wait()

    def hi_start(self, j):
        for i, p in enumerate(self.hi):
            p.copy(j, 1, self.hsem(j, i)).start(priority=HI)

    def hi_wait(self, j, n):
        for i, p in enumerate(self.hi):
            p.copy(j, n, self.hsem(0 if j is None else j, i)).wait()


def make_kernel(LA=39, HS=12, LA0=12, HS0=6, SL=20, checks=False, GSKIP=0, side=True, HE=None, T1=25, lag=True, SL2=23,
                SCHED=((4, "Z0"), (8, "S"), (12, "Z1")),
                TAIL=((56, 384, 64), (60, 448, 32), (64, 480, 32))):
    def kernel(xa_h, ckv_h, wqa_h, wuk_h, wuv_h, woa_h, xb_h, k_h, v_h, wqb_h, wob_h,
               out_ref,
               kbuf, vbuf, wqb_v, wqa_v, wuk_v, wuv_v, ckv_v, woa_v, wob_v, xa_v, xb_v,
               xs, qf_s, q_s, qm_s, s_s, m_s, l_s, acc_s, o_s, of_s, ol_s,
               qa_s, qabs_s, sa_s, ma_s, la_s, acca_s, ctxc_s, ctx_s, outb_s,
               lsem, hsem, esem, xsem, tsem):

        def kv(a, g):
            src, dst = (k_h, v_h)[a], (kbuf, vbuf)[a]
            s0 = g * 32 + 2 * PHI
            return _Block([_Part(src, dst, s0, SL, 0)],
                          [_Part(src, dst, s0 + SL, 32 - 2 * PHI - SL, SL),
                           _Part(src, dst, (g * 32 + 32) & (2 * NU - 1), 2 * PHI, 32 - 2 * PHI)],
                          lambda j, i: hsem.at[a * 8 + ((j >> 4) & 3) * 2 + i])

        first = _Block([_Part(wuv_h, wuv_v, 0, 8), _Part(wuk_h, wuk_v, 0, 8), _Part(wqa_h, wqa_v, 0, 8)],
                       [_Part(ckv_h, ckv_v, 0, 4), _Part(wqb_h, wqb_v, 0, 8)], lambda j, i: esem.at[i])
        second = _Block([_Part(ckv_h, ckv_v, 4, SL2)],
                        [_Part(ckv_h, ckv_v, 4 + SL2, 28 - SL2), _Part(wob_h, wob_v, 0, 8)], lambda j, i: esem.at[2 + i])
        tail_sem = {r // 8 + i: 3 + n for n, (_, r, w) in enumerate(TAIL) for i in range(w // 8)}
        last = _Block([_Part(woa_h, woa_v, 0, 5, width=512)], [_Part(woa_h, woa_v, 5, 3, width=512)],
                      lambda j, i: tsem.at[tail_sem.get(j, j // 16)], 64)

        def either(pos, lim, cur_fn, nxts, nxt_fn):
            if isinstance(pos, int):
                if pos < lim:
                    cur_fn()
                else:
                    assert not nxts
                return
            pl.when(pos < lim)(cur_fn)
            for cond, nxt in nxts:
                c = pos >= lim
                if cond is not None:
                    c = jnp.logical_and(c, cond)
                pl.when(c)(lambda nxt=nxt: nxt_fn(nxt))

        def point(cur, j, nxts, la, hs, h_next=None):
            if nxts is None or (h_next is not None and h_next < 0):
                cur.hi_start(j + hs)
            else:
                either(j + hs, cur.npts, lambda: cur.hi_start(j + hs), nxts,
                       lambda nxt: nxt.hi_start(j + hs - cur.npts if h_next is None else h_next))
            cur.lo_wait(j, lsem.at[j & 63])
            sem = lsem.at[(j + la) & 63]
            if nxts is None:
                cur.lo_start(j + la, sem)
            else:
                either(j + la, cur.npts, lambda: cur.lo_start(j + la, sem), nxts,
                       lambda nxt: nxt.lo_start(j + la - cur.npts, sem))

        def stream(cur, nxt, la, hs, extra=None):
            n1 = (cur.npts - max(la, hs)) // 4

            def body(m, c):
                for t in range(4):
                    point(cur, m * 4 + t, None, la, hs)
                if extra is not None:
                    extra(m)
                return c
            lax.fori_loop(0, n1, body, 0)

            def body2(j, c):
                point(cur, j, [(None, nxt)], la, hs)
                return c
            lax.fori_loop(n1 * 4, cur.npts, body2, 0)

        zeroed = [[xs, o_s, qa_s], [of_s, ctx_s, outb_s, ma_s], [ctxc_s.at[0], ctxc_s.at[1]], [ctxc_s.at[2], ctxc_s.at[3]]]
        xb_cp = pltpu.make_async_copy(xb_h, xb_v, xsem.at[0])
        xa_cp = pltpu.make_async_copy(xa_h, xa_v, xsem.at[1])
        assert LA0 == 2 * HS0
        for j in range(HS0):
            first.lo_start(2 * j, lsem.at[2 * j])
            first.hi_start(j)
            first.lo_start(2 * j + 1, lsem.at[2 * j + 1])
        xb_cp.start(priority=HI)
        xa_cp.start(priority=HI)
        for rs in zeroed:
            for r in rs:
                r[...] = jnp.zeros(r.shape, F32)

        stream(first, second, LA0, HS0)

        def deepen(j, c):
            second.lo_start(j, lsem.at[j])
            return c
        for j in range(HS0, HS):
            second.hi_start(j)
        lax.fori_loop(LA0, LA, deepen, 0)

        xb_cp.wait()
        xa_cp.wait()
        for s in range(4):
            xs[s, 0:B, :] = xa_v[:, s * 128:(s + 1) * 128].astype(F32)
            xs[4 + s, 0:B, :] = xb_v[:, s * 128:(s + 1) * 128].astype(F32)
        first.hi_wait(None, None)

        def qb_piece(m):
            @pl.when(jnp.logical_and((m & 7) == 3, m < 32))
            def _():
                hg = m >> 3
                x = jnp.concatenate([xs[4 + s] for s in range(4)], axis=-1).astype(BF16)
                w = wqb_v[:, :, pl.ds(pl.multiple_of(hg * 1024, 1024), 1024)].reshape(M, 1024)
                q = _dot(x, w)
                q = jnp.swapaxes(jnp.stack([q[:, h * D:(h + 1) * D] for h in range(8)]), 0, 1)
                for b in range(B):
                    qf_s[pl.ds(pl.multiple_of(b * H + hg * 8, 8), 8), :] = q[b]

        stream(second, kv(0, GSKIP), LA, HS, qb_piece)
        second.hi_wait(None, None)
        q_s[0:NU - PHI, :] = qf_s[PHI:NU, :]
        q_s[NU - PHI:NU, :] = qf_s[0:PHI, :]

        row = lax.broadcasted_iota(jnp.int32, (8, 8 * D), 0)
        col = lax.broadcasted_iota(jnp.int32, (8, 8 * D), 1) >> 7
        blk = row == col

        def tile(buf, z, hf, i):
            r = _mo(i * 128, 128)
            return jnp.concatenate([buf[z * 16 + 2 * n + hf, pl.ds(r, 128), :] for n in range(8)], axis=-1)

        def start_k(g, z):
            q = q_s[pl.ds(pl.multiple_of(g * 16 + z * 8, 8), 8), :]
            qm_s[z] = jnp.where(blk, jnp.concatenate([q] * 8, axis=-1), 0.0)
            m_s[z] = jnp.full((8, 128), -jnp.inf, F32)

        def qk(z, i):
            qm = qm_s[z].astype(BF16)
            m = m_s[z]
            for hf in range(2):
                s = _dot_nt(qm, tile(kbuf, z, hf, i))
                s_s[z, hf * 16 + i] = s
                m = jnp.maximum(m, s)
            m_s[z] = m

        def start_v(z):
            m_s[z] = jnp.broadcast_to(jnp.max(m_s[z], axis=-1, keepdims=True), (8, 128))
            l_s[z] = jnp.zeros((8, 128), F32)
            acc_s[z] = jnp.zeros((8, 8 * D), F32)

        def pv(z, i):
            l, acc = l_s[z], acc_s[z]
            for hf in range(2):
                p = jnp.exp((s_s[z, hf * 16 + i] - m_s[z]) * SCALE)
                l = l + p
                acc = acc + _dot(p.astype(BF16), tile(vbuf, z, hf, i))
            l_s[z] = l
            acc_s[z] = acc

        def finish_v(g, z):
            o = jnp.where(blk, acc_s[z], 0.0)
            o8 = o[:, 0:D]
            for i in range(1, 8):
                o8 = o8 + o[:, i * D:(i + 1) * D]
            o_s[pl.ds(pl.multiple_of(g * 16 + z * 8, 8), 8), :] = o8 / jnp.sum(l_s[z], axis=-1, keepdims=True)

        def per_heads(cond, u, fn):
            c = u >> 2
            for q in range(4):
                def heads(w_v, q=q):
                    w = w_v[pl.ds(c * 2, 2)].reshape(128, H, D)
                    return jnp.swapaxes(w[:, q * 8:(q + 1) * 8, :], 0, 1)
                pl.when(jnp.logical_and(cond, (u & 3) == q))(lambda q=q, heads=heads: fn(c, q, heads))

        def side_k(g, u):
            def a_q(c, q, heads):
                wt = heads(wqa_v)
                w = jnp.concatenate([wt[h] for h in range(8)], axis=-1)
                qa_s[:, q * 1024:(q + 1) * 1024] += _dot(xs[c].astype(BF16), w)
            per_heads(g == 0, u, a_q)

            ab = jnp.clip(g - 1, 0, B - 1)
            act = jnp.logical_and(g >= 1, g <= B)
            i = u & 7

            @pl.when(jnp.logical_and(act, u < 8))
            def _():
                qc = jnp.concatenate([qabs_s[s, ab] for s in range(4)], axis=-1).astype(BF16)
                s = _dot_nt(qc, ckv_v[ab * 8 + i])
                sa_s[i] = s
                m = jnp.maximum(jnp.maximum(s[:, 0:128], s[:, 128:256]), jnp.maximum(s[:, 256:384], s[:, 384:512]))
                ma_s[...] = jnp.where(u == 0, m, jnp.maximum(m, ma_s[...]))

            @pl.when(jnp.logical_and(act, u >= 8))
            def _():
                @pl.when(u == 8)
                def _():
                    ma_s[...] = jnp.broadcast_to(jnp.max(ma_s[...], axis=-1, keepdims=True), ma_s.shape)
                    la_s[...] = jnp.zeros(la_s.shape, F32)
                    acca_s[...] = jnp.zeros(acca_s.shape, F32)
                p = jnp.exp((sa_s[i] - jnp.concatenate([ma_s[...]] * 4, axis=-1)) * SCALE)
                la_s[...] += (p[:, 0:128] + p[:, 128:256]) + (p[:, 256:384] + p[:, 384:512])
                acca_s[...] += _dot(p.astype(BF16), ckv_v[ab * 8 + i])

                @pl.when(u == 15)
                def _():
                    c = acca_s[...] / jnp.sum(la_s[...], axis=-1, keepdims=True)
                    for s in range(4):
                        ctxc_s[s, ab] = c[:, s * 128:(s + 1) * 128]

            @pl.when(jnp.logical_and(g == NG - 1, u == 1))
            def _():
                of_s[PHI:NU, :] = o_s[0:NU - PHI, :]
                of_s[0:PHI, :] = o_s[NU - PHI:NU, :]
                t = jnp.swapaxes(of_s[...].reshape(8, H, D), 0, 1)
                for s in range(8):
                    ol_s[s] = jnp.concatenate([t[s * 4 + h] for h in range(4)], axis=-1)

        def side_v(g, u):
            def a_qabs(c, q, heads):
                wt = heads(wuk_v)
                qa = qa_s[:, q * 1024:(q + 1) * 1024].astype(BF16)
                t = jnp.stack([_dot_nt(qa[:, h * D:(h + 1) * D], wt[h]) for h in range(8)])
                qabs_s[c, :, q * 8:(q + 1) * 8, :] = jnp.swapaxes(t, 0, 1)
            per_heads(g == 0, u, a_qabs)

            def a_ctx(c, q, heads):
                wt = heads(wuv_v)
                x = jnp.swapaxes(ctxc_s[c, :, q * 8:(q + 1) * 8, :], 0, 1).astype(BF16)
                ctx_s[:, q * 1024:(q + 1) * 1024] += jnp.concatenate([_dot(x[h], wt[h]) for h in range(8)], axis=-1)
            per_heads(g == B + 1, u, a_ctx)

            @pl.when(jnp.logical_and(g == NG - 1, u < 8))
            def _():
                outb_s[...] += _dot(ol_s[u & 7].astype(BF16), wob_v[u & 7])

        def work(a, g, z, i):
            if z == 1:
                kv(a, g).hi_wait(i * 16, 16)
            (pv if a else qk)(z, i)

        def wrap_up(a, g, z):
            work(a, g, z, 15)
            if a == 0:
                start_v(z)
            else:
                finish_v(g, z)

        def phase(a, g):
            cur = kv(a, g)
            if a == 0:
                nxts = [(None, kv(1, g))]
            else:
                nxts = [(g < NG - 1, kv(0, jnp.minimum(g + 1, NG - 1))), (g == NG - 1, last)]
            sched = dict(SCHED)

            def group(u, c):
                for t in range(16):
                    point(cur, u * 16 + t, nxts, LA, HS, h_next=t + HS - 16)
                    item = sched.get(t + 1)
                    if item == "S":
                        if side:
                            (side_v if a else side_k)(g, u)
                    elif item is not None:
                        z = int(item[1])
                        pl.when(u > 0)(lambda: work(a, g, z, u - 1))

                        @pl.when(u == 0)
                        def _():
                            if a == 1:
                                wrap_up(0, g, z)
                            else:
                                pl.when(g > GSKIP)(lambda: wrap_up(1, g - 1, z))
                                start_k(g, z)
                return c
            lax.fori_loop(0, 16, group, 0)

        def body(g, c):
            phase(0, g)
            phase(1, g)
            return c
        lax.fori_loop(GSKIP, NG, body, 0)

        def lhs(streams, r, n):
            return jnp.concatenate([ctx_s[:, s * 512 + r:s * 512 + r + n] for s in streams], axis=-1).astype(BF16)

        def rhs(streams, r, n):
            return jnp.concatenate([woa_v[s, r:r + n, :] for s in streams], axis=0)

        def last_share(z):
            units = [((NG - 1) * 16 + PHI + z * 8 + i) % NU for i in range(8)]
            o = jnp.where(blk, acc_s[z] / jnp.sum(l_s[z], axis=-1, keepdims=True), 0.0)
            o = jnp.broadcast_to(jnp.sum(o, axis=0, keepdims=True), (8, 8 * D))
            n0 = sum(n // H == units[0] // H for n in units)
            o = jnp.where(row == jnp.where(col < n0, units[0] // H, units[-1] // H), o, 0.0)
            w = jnp.concatenate([wob_v[n % H // 4, (n % 4) * D:(n % 4 + 1) * D, :] for n in units], axis=0)
            return _dot(o.astype(BF16), w)

        full = {24: (0, 0), 29: (0, 1), 34: (1, 0), 39: (1, 1), 48: (2, 0), 52: (2, 1)}
        tail = {t: (r, n) for t, r, n in TAIL}
        tail_lhs = {}
        acc = None
        hj = HS
        he = HS if HE is None else HE
        for t in range(1, last.npts + 1):
            if hj < last.npts and not (t > T1 and hj - (t - 1) > he and t % 2 == 0):
                last.hi_start(hj)
                hj += 1
            last.lo_wait(t - 1, lsem.at[t - 1])
            if t - 1 + LA < last.npts:
                last.lo_start(t - 1 + LA, lsem.at[t - 1 + LA])
            if t in (2, 6):
                work(1, NG - 1, t // 4, 15)
            if t == 10:
                outb_s[...] += last_share(0)
            if t == 17:
                out_ref[:, M:] = (outb_s[...] + last_share(1))[0:B, :].astype(out_ref.dtype)
            if t == 43:
                tail_lhs = {tt: lhs(range(8), r, n) for tt, (r, n) in tail.items()}
            if t in full:
                i, hf = full[t]
                assert (i + 1) * 16 <= t
                if hf:
                    last.hi_wait(i * 16, 16)
                ss = range(hf * 4, hf * 4 + 4)
                d = _dot(lhs(ss, i * 128, 128), rhs(ss, i * 128, 128))
                acc = d if acc is None else acc + d
            if t in tail:
                r, n = tail[t]
                assert r + n <= t * 8
                last.hi_wait(r // 8, n // 8)
                acc = acc + _dot(tail_lhs[t], rhs(range(8), r, n))
        assert hj == last.npts
        out_ref[:, :M] = acc[0:B, :].astype(out_ref.dtype)

    scratch = [
        pltpu.VMEM((32, 2048, D), BF16), pltpu.VMEM((32, 2048, D), BF16),
        pltpu.VMEM((8, 64, H * D), BF16),
        pltpu.VMEM((8, 2048, D), BF16), pltpu.VMEM((8, 2048, D), BF16), pltpu.VMEM((8, 2048, D), BF16),
        pltpu.VMEM((32, 512, DC), BF16),
        pltpu.VMEM((8, 512, M), BF16), pltpu.VMEM((8, 512, M), BF16),
        pltpu.VMEM((B, M), BF16), pltpu.VMEM((B, M), BF16),
        pltpu.VMEM((8, 8, 128), F32),
        pltpu.VMEM((NU, D), F32),
        pltpu.VMEM((NU, D), F32),
        pltpu.VMEM((2, 8, 8 * D), F32),
        pltpu.VMEM((2, 32, 8, 128), F32),
        pltpu.VMEM((2, 8, 128), F32),
        pltpu.VMEM((2, 8, 128), F32),
        pltpu.VMEM((2, 8, 8 * D), F32),
        pltpu.VMEM((NU, D), F32),
        pltpu.VMEM((8 * H, D), F32),
        pltpu.VMEM((8, 8, 512), F32),
        pltpu.VMEM((8, H * D), F32),
        pltpu.VMEM((4, 8, H, 128), F32),
        pltpu.VMEM((8, H, 512), F32),
        pltpu.VMEM((H, 128), F32),
        pltpu.VMEM((H, 128), F32),
        pltpu.VMEM((H, DC), F32),
        pltpu.VMEM((4, 8, H, 128), F32),
        pltpu.VMEM((8, H * D), F32),
        pltpu.VMEM((8, M), F32),
        pltpu.SemaphoreType.DMA((64,)),
        pltpu.SemaphoreType.DMA((16,)),
        pltpu.SemaphoreType.DMA((4,)),
        pltpu.SemaphoreType.DMA((2,)),
        pltpu.SemaphoreType.DMA((3 + len(TAIL),)),
    ]

    @jax.jit
    def fn(A_x, A_c_kv, A_w_q, A_w_uk, A_w_uv, A_w_o, B_x, B_k_cache, B_v_cache, B_wq, B_wo):
        out = pl.pallas_call(
            kernel,
            in_specs=[pl.BlockSpec(memory_space=pl.ANY)] * 11,
            out_specs=pl.BlockSpec(memory_space=pltpu.VMEM),
            out_shape=jax.ShapeDtypeStruct((B, 2 * M), BF16),
            scratch_shapes=scratch,
            compiler_params=pltpu.CompilerParams(vmem_limit_bytes=100 * 1024 * 1024, disable_bounds_checks=not checks,
                                                 disable_semaphore_checks=not checks),
            name="fused_decode",
        )(A_x.reshape(B, M), A_c_kv.reshape(32, 512, DC), A_w_q.reshape(8, 2048, D), A_w_uk.reshape(8, 2048, D),
          A_w_uv.reshape(8, 2048, D), A_w_o.reshape(8, 512, M), B_x.reshape(B, M),
          B_k_cache.reshape(2 * NU, 2048, D), B_v_cache.reshape(2 * NU, 2048, D),
          B_wq.reshape(8, 64, H * D), B_wo.reshape(8, 512, M))
        return out.reshape(B, 1, 2 * M)

    return fn


_fn = make_kernel()


@jax.jit
def pallas_concat_heads__compressed_kv_cla__mha_block_cached__decode_kernel(
    A_x: jax.Array,
    A_c_kv: jax.Array,
    A_w_q: jax.Array,
    A_w_uk: jax.Array,
    A_w_uv: jax.Array,
    A_w_o: jax.Array,
    B_x: jax.Array,
    B_k_cache: jax.Array,
    B_v_cache: jax.Array,
    B_wq: jax.Array,
    B_wo: jax.Array,
):
    return _fn(A_x, A_c_kv, A_w_q, A_w_uk, A_w_uv, A_w_o, B_x, B_k_cache, B_v_cache, B_wq, B_wo)
```

```python
import jax
import jax.numpy as jnp
from jax import lax
import jax.experimental.pallas as pl
import jax.experimental.pallas.tpu as pltpu

B, H, SK, D, M = 4, 32, 4096, 128, 512
DC = 512
NU = B * H
NG = NU // 16
ROLL = 14
F32 = jnp.float32
BF16 = jnp.bfloat16
LO, HI = 1, 0
SCALE = D ** -0.5
ALL = slice(None)


def _dot(a, b):
    return jnp.dot(a, b, preferred_element_type=F32)


def _dot_nt(a, b):
    return lax.dot_general(a, b, (((1,), (1,)), ((), ())), preferred_element_type=F32)


def _mo(x, n):
    return x if isinstance(x, int) else pl.multiple_of(x, n)


class _Part:
    cond = None

    def __init__(self, src, dst, s0, n, d0=None, width=128):
        self.src = src.at[pl.ds(s0, n)]
        self.dst = dst.at[pl.ds(s0 if d0 is None else d0, n)]
        self.lg = (src.shape[-1] // width).bit_length() - 1
        self.width = width

    def copy(self, j, n, sem):
        if j is None:
            idx = (ALL,)
        elif self.lg == 0:
            idx = (ALL, pl.ds(_mo(j * 8, 8), n * 8))
        else:
            assert n == 1
            idx = (ALL, pl.ds(_mo((j >> self.lg) * 8, 8), 8),
                   pl.ds(_mo((j & ((1 << self.lg) - 1)) * self.width, 128), self.width))
        return pltpu.make_async_copy(self.src.at[idx], self.dst.at[idx], sem)


class _Block:
    def __init__(self, lo, hi, hsem, npts=256):
        self.lo, self.hi, self.hsem, self.npts = lo, hi, hsem, npts

    def lo_start(self, j, sem):
        for p in self.lo:
            p.copy(j, 1, sem).start(priority=LO)

    def lo_wait(self, j, sem):
        for p in self.lo:
            p.copy(j, 1, sem).wait()

    def _hi(self, fn):
        for i, p in enumerate(self.hi):
            if p.cond is None:
                fn(i, p)
            else:
                pl.when(p.cond)(lambda: fn(i, p))

    def hi_start(self, j):
        self._hi(lambda i, p: p.copy(j, 1, self.hsem(j, i)).start(priority=HI))

    def hi_wait(self, j, n):
        self._hi(lambda i, p: p.copy(j, n, self.hsem(0 if j is None else j, i)).wait())


def make_kernel(LA=39, HS=12, LA0=16, HS0=8, SL=20, SL2=18, checks=False,
                SCHED=((4, "Z0"), (8, "S"), (12, "Z1")),
                FULL=((22, 0, 0), (26, 0, 1), (32, 1, 0), (36, 1, 1)), TL=29,
                TAIL=((41, 256, 64), (48, 320, 64), (56, 384, 64), (60, 448, 32), (64, 480, 32))):
    def kernel(xa_h, ckv_h, wqa_h, wuk_h, wuv_h, woa_h, xb_h, k_h, v_h, wqb_h, wob_h,
               out_ref,
               kbuf, vbuf, wqb_v, wqa_v, wuk_v, wuv_v, ckv_v, woa_v, wob_v, xa_v, xb_v,
               xs, qf_s, q_s, qm_s, s_s, m_s, l_s, acc_s, o_s, of_s, ol_s,
               qa_s, qabs_s, sa_s, ma_s, la_s, acca_s, ctxc_s, ctx_s, outb_s,
               lsem, hsem, esem, xsem, tsem):

        def kv(a, g, wraps=True):
            src, dst = (k_h, v_h)[a], (kbuf, vbuf)[a]
            short = _Part(src, dst, 2 * NU - 2 * ROLL + SL, 2 * ROLL - SL, SL)
            if isinstance(g, int):
                hi = [short if g == 0 else _Part(src, dst, g * 32 - 2 * ROLL + SL, 32 - SL, SL)]
            else:
                hi = [_Part(src, dst, jnp.maximum(g * 32 - 2 * ROLL + SL, 0), 32 - SL, SL)]
                if wraps:
                    hi[0].cond, short.cond = g > 0, g == 0
                    hi.append(short)
            return _Block([_Part(src, dst, (g * 32 - 2 * ROLL) & (2 * NU - 1), SL, 0)], hi,
                          lambda j, i: hsem.at[a * 4 + ((j >> 4) & 3)])

        pre = [
            _Block([_Part(wqb_h, wqb_v, 0, 8), _Part(wob_h, wob_v, 0, 8)],
                   [_Part(v_h, vbuf, 0, 4, 2 * ROLL), _Part(k_h, kbuf, 0, 4, 2 * ROLL)], lambda j, i: esem.at[i]),
            _Block([_Part(wuk_h, wuk_v, 0, 8), _Part(wqa_h, wqa_v, 0, 8), _Part(ckv_h, ckv_v, 0, 4)],
                   [_Part(wuv_h, wuv_v, 0, 8)], lambda j, i: esem.at[2]),
            _Block([_Part(ckv_h, ckv_v, 4, SL2)], [_Part(ckv_h, ckv_v, 4 + SL2, 28 - SL2)], lambda j, i: esem.at[3]),
        ]
        tail_sem = {r // 8 + i: 3 + n for n, (_, r, w) in enumerate(TAIL) for i in range(w // 8)}
        last = _Block([_Part(woa_h, woa_v, 0, 5, width=512)], [_Part(woa_h, woa_v, 5, 3, width=512)],
                      lambda j, i: tsem.at[tail_sem.get(j, j // 16)], 64)

        def either(pos, lim, cur_fn, nxts, nxt_fn):
            if isinstance(pos, int):
                if pos < lim:
                    cur_fn()
                else:
                    assert not nxts
                return
            pl.when(pos < lim)(cur_fn)
            for cond, nxt in nxts:
                c = pos >= lim
                if cond is not None:
                    c = jnp.logical_and(c, cond)
                pl.when(c)(lambda nxt=nxt: nxt_fn(nxt))

        def point(cur, j, nxts, la, hs, h_next=None):
            if nxts is None or (h_next is not None and h_next < 0):
                cur.hi_start(j + hs)
            else:
                either(j + hs, cur.npts, lambda: cur.hi_start(j + hs), nxts,
                       lambda nxt: nxt.hi_start(j + hs - cur.npts if h_next is None else h_next))
            cur.lo_wait(j, lsem.at[j & 63])
            sem = lsem.at[(j + la) & 63]
            if nxts is None:
                cur.lo_start(j + la, sem)
            else:
                either(j + la, cur.npts, lambda: cur.lo_start(j + la, sem), nxts,
                       lambda nxt: nxt.lo_start(j + la - cur.npts, sem))

        def stream(cur, nxt, la, hs, extra=None):
            n1 = (cur.npts - max(la, hs)) // 4

            def body(m, c):
                for t in range(4):
                    point(cur, m * 4 + t, None, la, hs)
                if extra is not None:
                    extra(m)
                return c
            lax.fori_loop(0, n1, body, 0)

            def body2(j, c):
                point(cur, j, [(None, nxt)], la, hs)
                return c
            lax.fori_loop(n1 * 4, cur.npts, body2, 0)

        xb_cp = pltpu.make_async_copy(xb_h, xb_v, xsem.at[0])
        xa_cp = pltpu.make_async_copy(xa_h, xa_v, xsem.at[1])
        for j in range(LA0):
            pre[0].lo_start(j, lsem.at[j])
            if j % 2 == 0 and j // 2 < HS0:
                pre[0].hi_start(j // 2)
        assert LA0 + 1 >= 2 * HS0
        xb_cp.start(priority=HI)
        xa_cp.start(priority=HI)
        for r in (xs, o_s, qa_s, of_s, ctx_s, outb_s, ma_s, ctxc_s):
            r[...] = jnp.zeros(r.shape, F32)

        stream(pre[0], pre[1], LA0, HS0)
        stream(pre[1], pre[2], LA0, HS0)

        def deepen(j, c):
            pre[2].lo_start(j, lsem.at[j])

            @pl.when(j >= LA - (HS - HS0))
            def _():
                pre[2].hi_start(j - (LA - HS))
            return c
        lax.fori_loop(LA0, LA, deepen, 0)

        pre[0].hi_wait(None, None)
        pre[1].hi_wait(None, None)
        xb_cp.wait()
        xa_cp.wait()
        for s in range(4):
            xs[s, 0:B, :] = xa_v[:, s * 128:(s + 1) * 128].astype(F32)
            xs[4 + s, 0:B, :] = xb_v[:, s * 128:(s + 1) * 128].astype(F32)

        def qb_piece(m):
            @pl.when(jnp.logical_and((m & 7) == 3, m < 32))
            def _():
                hg = m >> 3
                x = jnp.concatenate([xs[4 + s] for s in range(4)], axis=-1).astype(BF16)
                w = wqb_v[:, :, pl.ds(pl.multiple_of(hg * 1024, 1024), 1024)].reshape(M, 1024)
                q = _dot(x, w)
                q = jnp.swapaxes(jnp.stack([q[:, h * D:(h + 1) * D] for h in range(8)]), 0, 1)
                for b in range(B):
                    qf_s[pl.ds(pl.multiple_of(b * H + hg * 8, 8), 8), :] = q[b]

        stream(pre[2], kv(0, 0), LA, HS, qb_piece)
        pre[2].hi_wait(None, None)
        q_s[ROLL:NU, :] = qf_s[0:NU - ROLL, :]
        q_s[0:ROLL, :] = qf_s[NU - ROLL:NU, :]

        row = lax.broadcasted_iota(jnp.int32, (8, 8 * D), 0)
        blk = row == (lax.broadcasted_iota(jnp.int32, (8, 8 * D), 1) >> 7)

        def tile(buf, z, hf, i):
            r = _mo(i * 128, 128)
            return jnp.concatenate([buf[z * 16 + 2 * n + hf, pl.ds(r, 128), :] for n in range(8)], axis=-1)

        def start_k(g, z):
            q = q_s[pl.ds(pl.multiple_of(g * 16 + z * 8, 8), 8), :]
            qm_s[z] = jnp.where(blk, jnp.concatenate([q] * 8, axis=-1), 0.0)
            m_s[z] = jnp.full((8, 128), -jnp.inf, F32)

        def qk(z, i):
            qm = qm_s[z].astype(BF16)
            m = m_s[z]
            for hf in range(2):
                s = _dot_nt(qm, tile(kbuf, z, hf, i))
                s_s[z, hf * 16 + i] = s
                m = jnp.maximum(m, s)
            m_s[z] = m

        def start_v(z):
            m_s[z] = jnp.broadcast_to(jnp.max(m_s[z], axis=-1, keepdims=True), (8, 128))
            l_s[z] = jnp.zeros((8, 128), F32)
            acc_s[z] = jnp.zeros((8, 8 * D), F32)

        def pv(z, i):
            l, acc = l_s[z], acc_s[z]
            for hf in range(2):
                p = jnp.exp((s_s[z, hf * 16 + i] - m_s[z]) * SCALE)
                l = l + p
                acc = acc + _dot(p.astype(BF16), tile(vbuf, z, hf, i))
            l_s[z] = l
            acc_s[z] = acc

        def finish_v(g, z):
            o = jnp.where(blk, acc_s[z], 0.0)
            o8 = o[:, 0:D]
            for i in range(1, 8):
                o8 = o8 + o[:, i * D:(i + 1) * D]
            o_s[pl.ds(pl.multiple_of(g * 16 + z * 8, 8), 8), :] = o8 / jnp.sum(l_s[z], axis=-1, keepdims=True)

        def per_heads(cond, u, fn):
            c = u >> 2
            for q in range(4):
                def heads(w_v, q=q):
                    w = w_v[pl.ds(c * 2, 2)].reshape(128, H, D)
                    return jnp.swapaxes(w[:, q * 8:(q + 1) * 8, :], 0, 1)
                pl.when(jnp.logical_and(cond, (u & 3) == q))(lambda q=q, heads=heads: fn(c, q, heads))

        def side_k(g, u):
            def a_q(c, q, heads):
                wt = heads(wqa_v)
                w = jnp.concatenate([wt[h] for h in range(8)], axis=-1)
                qa_s[:, q * 1024:(q + 1) * 1024] += _dot(xs[c].astype(BF16), w)
            per_heads(g == 0, u, a_q)

            ab = jnp.clip(g - 1, 0, B - 1)
            act = jnp.logical_and(g >= 1, g <= B)
            i = u & 7

            @pl.when(jnp.logical_and(act, u < 8))
            def _():
                qc = jnp.concatenate([qabs_s[s, ab] for s in range(4)], axis=-1).astype(BF16)
                s = _dot_nt(qc, ckv_v[ab * 8 + i])
                sa_s[i] = s
                m = jnp.maximum(jnp.maximum(s[:, 0:128], s[:, 128:256]), jnp.maximum(s[:, 256:384], s[:, 384:512]))
                ma_s[...] = jnp.where(u == 0, m, jnp.maximum(m, ma_s[...]))

            @pl.when(jnp.logical_and(act, u >= 8))
            def _():
                @pl.when(u == 8)
                def _():
                    ma_s[...] = jnp.broadcast_to(jnp.max(ma_s[...], axis=-1, keepdims=True), ma_s.shape)
                    la_s[...] = jnp.zeros(la_s.shape, F32)
                    acca_s[...] = jnp.zeros(acca_s.shape, F32)
                p = jnp.exp((sa_s[i] - jnp.concatenate([ma_s[...]] * 4, axis=-1)) * SCALE)
                la_s[...] += (p[:, 0:128] + p[:, 128:256]) + (p[:, 256:384] + p[:, 384:512])
                acca_s[...] += _dot(p.astype(BF16), ckv_v[ab * 8 + i])

                @pl.when(u == 15)
                def _():
                    c = acca_s[...] / jnp.sum(la_s[...], axis=-1, keepdims=True)
                    for s in range(4):
                        ctxc_s[s, ab] = c[:, s * 128:(s + 1) * 128]

            @pl.when(jnp.logical_and(g == NG - 1, u == 1))
            def _():
                of_s[0:NU - ROLL, :] = o_s[ROLL:NU, :]
                of_s[NU - ROLL:NU, :] = o_s[0:ROLL, :]
                t = jnp.swapaxes(of_s[...].reshape(8, H, D), 0, 1)
                for s in range(8):
                    ol_s[s] = jnp.concatenate([t[s * 4 + h] for h in range(4)], axis=-1)

        def side_v(g, u):
            def a_qabs(c, q, heads):
                wt = heads(wuk_v)
                qa = qa_s[:, q * 1024:(q + 1) * 1024].astype(BF16)
                t = jnp.stack([_dot_nt(qa[:, h * D:(h + 1) * D], wt[h]) for h in range(8)])
                qabs_s[c, :, q * 8:(q + 1) * 8, :] = jnp.swapaxes(t, 0, 1)
            per_heads(g == 0, u, a_qabs)

            def a_ctx(c, q, heads):
                wt = heads(wuv_v)
                x = jnp.swapaxes(ctxc_s[c, :, q * 8:(q + 1) * 8, :], 0, 1).astype(BF16)
                ctx_s[:, q * 1024:(q + 1) * 1024] += jnp.concatenate([_dot(x[h], wt[h]) for h in range(8)], axis=-1)
            per_heads(g == B + 1, u, a_ctx)

            @pl.when(jnp.logical_and(g == NG - 1, u < 8))
            def _():
                outb_s[...] += _dot(ol_s[u & 7].astype(BF16), wob_v[u & 7])

        def work(a, g, z, i):
            if z == 1:
                kv(a, g).hi_wait(i * 16, 16)
            (pv if a else qk)(z, i)

        def wrap_up(a, g, z):
            work(a, g, z, 15)
            if a == 0:
                start_v(z)
            else:
                finish_v(g, z)

        def phase(a, g):
            cur = kv(a, g)
            if a == 0:
                nxts = [(None, kv(1, g))]
            else:
                nxts = [(g < NG - 1, kv(0, jnp.minimum(g + 1, NG - 1), False)), (g == NG - 1, last)]
            sched = dict(SCHED)

            def group(u, c):
                for t in range(16):
                    point(cur, u * 16 + t, nxts, LA, HS, h_next=t + HS - 16)
                    item = sched.get(t + 1)
                    if item == "S":
                        (side_v if a else side_k)(g, u)
                    elif item is not None:
                        z = int(item[1])
                        pl.when(u > 0)(lambda: work(a, g, z, u - 1))

                        @pl.when(u == 0)
                        def _():
                            if a == 1:
                                wrap_up(0, g, z)
                            else:
                                pl.when(g > 0)(lambda: wrap_up(1, g - 1, z))
                                start_k(g, z)
                return c
            lax.fori_loop(0, 16, group, 0)

        def body(g, c):
            phase(0, g)
            phase(1, g)
            return c
        lax.fori_loop(0, NG, body, 0)

        def lhs(streams, r, n):
            return jnp.concatenate([ctx_s[:, s * 512 + r:s * 512 + r + n] for s in streams], axis=-1).astype(BF16)

        def rhs(streams, r, n):
            return jnp.concatenate([woa_v[s, r:r + n, :] for s in streams], axis=0)

        def last_share(z):
            units = [(NG - 1) * 16 - ROLL + z * 8 + i for i in range(8)]
            assert units[0] // H == units[-1] // H
            o = jnp.where(blk, acc_s[z] / jnp.sum(l_s[z], axis=-1, keepdims=True), 0.0)
            o = jnp.broadcast_to(jnp.sum(o, axis=0, keepdims=True), (8, 8 * D))
            o = jnp.where(row == units[0] // H, o, 0.0)
            w = jnp.concatenate([wob_v[n % H // 4, (n % 4) * D:(n % 4 + 1) * D, :] for n in units], axis=0)
            return _dot(o.astype(BF16), w)

        full = {t: (i, hf) for t, i, hf in FULL}
        tail = {t: (r, n) for t, r, n in TAIL}
        tail_lhs = {}
        acc = None
        for t in range(1, last.npts + 1):
            point(last, t - 1, [], LA, HS)
            if t in (2, 6):
                work(1, NG - 1, t // 4, 15)
            if t == 10:
                outb_s[...] += last_share(0)
            if t == 17:
                out_ref[:, M:] = (outb_s[...] + last_share(1))[0:B, :].astype(out_ref.dtype)
            if t == TL:
                tail_lhs = {tt: lhs(range(8), r, n) for tt, (r, n) in tail.items()}
            if t in full:
                i, hf = full[t]
                assert (i + 1) * 16 <= t
                if hf:
                    last.hi_wait(i * 16, 16)
                ss = range(hf * 4, hf * 4 + 4)
                d = _dot(lhs(ss, i * 128, 128), rhs(ss, i * 128, 128))
                acc = d if acc is None else acc + d
            if t in tail:
                r, n = tail[t]
                assert r + n <= t * 8
                last.hi_wait(r // 8, n // 8)
                acc = acc + _dot(tail_lhs[t], rhs(range(8), r, n))
        out_ref[:, :M] = acc[0:B, :].astype(out_ref.dtype)

    scratch = [
        pltpu.VMEM((32, 2048, D), BF16), pltpu.VMEM((32, 2048, D), BF16),
        pltpu.VMEM((8, 64, H * D), BF16),
        pltpu.VMEM((8, 2048, D), BF16), pltpu.VMEM((8, 2048, D), BF16), pltpu.VMEM((8, 2048, D), BF16),
        pltpu.VMEM((32, 512, DC), BF16),
        pltpu.VMEM((8, 512, M), BF16), pltpu.VMEM((8, 512, M), BF16),
        pltpu.VMEM((B, M), BF16), pltpu.VMEM((B, M), BF16),
        pltpu.VMEM((8, 8, 128), F32),
        pltpu.VMEM((NU, D), F32),
        pltpu.VMEM((NU, D), F32),
        pltpu.VMEM((2, 8, 8 * D), F32),
        pltpu.VMEM((2, 32, 8, 128), F32),
        pltpu.VMEM((2, 8, 128), F32),
        pltpu.VMEM((2, 8, 128), F32),
        pltpu.VMEM((2, 8, 8 * D), F32),
        pltpu.VMEM((NU, D), F32),
        pltpu.VMEM((8 * H, D), F32),
        pltpu.VMEM((8, 8, 512), F32),
        pltpu.VMEM((8, H * D), F32),
        pltpu.VMEM((4, 8, H, 128), F32),
        pltpu.VMEM((8, H, 512), F32),
        pltpu.VMEM((H, 128), F32),
        pltpu.VMEM((H, 128), F32),
        pltpu.VMEM((H, DC), F32),
        pltpu.VMEM((4, 8, H, 128), F32),
        pltpu.VMEM((8, H * D), F32),
        pltpu.VMEM((8, M), F32),
        pltpu.SemaphoreType.DMA((64,)),
        pltpu.SemaphoreType.DMA((8,)),
        pltpu.SemaphoreType.DMA((4,)),
        pltpu.SemaphoreType.DMA((2,)),
        pltpu.SemaphoreType.DMA((3 + len(TAIL),)),
    ]

    @jax.jit
    def fn(A_x, A_c_kv, A_w_q, A_w_uk, A_w_uv, A_w_o, B_x, B_k_cache, B_v_cache, B_wq, B_wo):
        out = pl.pallas_call(
            kernel,
            in_specs=[pl.BlockSpec(memory_space=pl.ANY)] * 11,
            out_specs=pl.BlockSpec(memory_space=pltpu.VMEM),
            out_shape=jax.ShapeDtypeStruct((B, 2 * M), BF16),
            scratch_shapes=scratch,
            compiler_params=pltpu.CompilerParams(vmem_limit_bytes=100 * 1024 * 1024, disable_bounds_checks=not checks,
                                                 disable_semaphore_checks=not checks),
            name="fused_decode",
        )(A_x.reshape(B, M), A_c_kv.reshape(32, 512, DC), A_w_q.reshape(8, 2048, D), A_w_uk.reshape(8, 2048, D),
          A_w_uv.reshape(8, 2048, D), A_w_o.reshape(8, 512, M), B_x.reshape(B, M),
          B_k_cache.reshape(2 * NU, 2048, D), B_v_cache.reshape(2 * NU, 2048, D),
          B_wq.reshape(8, 64, H * D), B_wo.reshape(8, 512, M))
        return out.reshape(B, 1, 2 * M)

    return fn


_fn = make_kernel()


@jax.jit
def pallas_concat_heads__compressed_kv_cla__mha_block_cached__decode_kernel(
    A_x: jax.Array,
    A_c_kv: jax.Array,
    A_w_q: jax.Array,
    A_w_uk: jax.Array,
    A_w_uv: jax.Array,
    A_w_o: jax.Array,
    B_x: jax.Array,
    B_k_cache: jax.Array,
    B_v_cache: jax.Array,
    B_wq: jax.Array,
    B_wo: jax.Array,
):
    return _fn(A_x, A_c_kv, A_w_q, A_w_uk, A_w_uv, A_w_o, B_x, B_k_cache, B_v_cache, B_wq, B_wo)
```
